```python
import jax
import jax.numpy as jnp

def _softmax(x, axis=-1):
    return jax.nn.softmax(x, axis=axis)
def _gelu(x):
    return jax.nn.gelu(x, approximate=True)
def _silu(x):
    return jax.nn.silu(x)
def _sigmoid(x):
    return jax.nn.sigmoid(x)
def _layernorm(x, axis=-1, eps=1e-5):
    m = jnp.mean(x, axis=axis, keepdims=True)
    v = jnp.var(x, axis=axis, keepdims=True)
    return (x - m) / jnp.sqrt(v + eps)
def _scatter_add(tgt, idx, src, axis=0):
    return tgt.at[idx].add(src)
def _segment_sum(src, seg, n):
    return jax.ops.segment_sum(src, seg, n)
class _Rng:
    def __init__(self, key):
        self._k = key
    def _next(self):
        self._k, sub = jax.random.split(self._k)
        return sub
    def normal(self, shape):
        return jax.random.normal(self._next(), shape, dtype=jnp.bfloat16)
    def randint(self, lo, hi, shape):
        return jax.random.randint(self._next(), shape, lo, hi, dtype=jnp.int32)
    def uniform(self, shape, lo=0.0, hi=1.0):
        return jax.random.uniform(self._next(), shape, jnp.bfloat16, lo, hi)
    def permutation(self, n):
        return jax.random.permutation(self._next(), n)


kernel_name = 'interleave_layers__sliding_local_dilated__glu_gated_swiglu__prompt'

def setup_inputs():
    _rng = _Rng(jax.random.key(int.from_bytes(__import__("os").urandom(4), "little")))
    _w = (lambda a: (lambda t: t.astype(jnp.bfloat16) if jnp.issubdtype(t.dtype, jnp.floating) else t)(jnp.asarray(a)))
    def _A_setup():
        B, S, D = 1, 2048, 1024
        return {
            "x": _w((lambda *s: _rng.normal(s) * 0.05)(B, S, D)),
            "wqkv": _w((lambda *s: _rng.normal(s) * 0.05)(D, 3 * D)),
            "wo": _w((lambda *s: _rng.normal(s) * 0.05)(D, D)),
        }
    _A_in = _A_setup()

    def _B_setup():
        B, S, D, F = 1, 2048, 1024, 3584
        return {
            "x": _w((lambda *s: _rng.normal(s) * 0.05)(B, S, D)),
            "w1": _w((lambda *s: _rng.normal(s) * 0.05)(D, F) * (2.0 / D) ** 0.5),
            "w3": _w((lambda *s: _rng.normal(s) * 0.05)(D, F) * (2.0 / D) ** 0.5),
            "w2": _w((lambda *s: _rng.normal(s) * 0.05)(F, D) * (2.0 / F) ** 0.5),
        }
    _B_in = _B_setup()

    return {
        "A_x": _A_in["x"],
        "A_wqkv": _A_in["wqkv"],
        "A_wo": _A_in["wo"],
        "B_x": _B_in["x"],
        "B_w1": _B_in["w1"],
        "B_w3": _B_in["w3"],
        "B_w2": _B_in["w2"],
    }

def reference(A_x, A_wqkv, A_wo, B_x, B_w1, B_w3, B_w2):
    def _A_ref(x, wqkv, wo):
        B, S, D = x.shape
        H = 32; Dh = D // H
        W, dil = 8, 2
        qkv = (lambda x, *d: x.transpose(*d))((x @ wqkv).reshape(B, S, 3, H, Dh), 2, 0, 3, 1, 4)
        q, k, v = qkv[0], qkv[1], qkv[2]
        scale = Dh ** -0.5
        pos = jnp.arange(S)
        off = jnp.arange(W) * dil
        idx = pos[:, None] - off[None, :]
        mask = idx >= 0
        idx_c = jnp.where(mask, idx, 0).reshape(-1)
        kg = k[:, :, idx_c, :].reshape(B, H, S, W, Dh)
        vg = v[:, :, idx_c, :].reshape(B, H, S, W, Dh)
        logits = jnp.einsum("bhsd,bhswd->bhsw", q, kg) * scale
        logits = jnp.where(mask[None, None, :, :], logits, -1e9)
        attn = _softmax(logits, axis=-1)
        o = jnp.einsum("bhsw,bhswd->bhsd", attn, vg)
        return (lambda x, *d: x.transpose(*d))(o, 0, 2, 1, 3).reshape(B, S, D) @ wo

    def _B_ref(x, w1, w3, w2):
        gate = jnp.einsum("bsd,df->bsf", x, w1)
        up = jnp.einsum("bsd,df->bsf", x, w3)
        h = _silu(gate) * up
        out = jnp.einsum("bsf,fd->bsd", h, w2)
        return out

    x = A_x
    x = x + _A_ref(_layernorm(x, axis=-1), A_wqkv, A_wo)
    x = x + _B_ref(_layernorm(x, axis=-1), B_w1, B_w3, B_w2)
    x = x + _A_ref(_layernorm(x, axis=-1), A_wqkv, A_wo)
    x = x + _B_ref(_layernorm(x, axis=-1), B_w1, B_w3, B_w2)
    return x
```

```python
import functools
import jax
import jax.numpy as jnp
from jax.experimental import pallas as pl
from jax.experimental.pallas import tpu as pltpu

S, D, F = 2048, 1024, 3584
H, DH, W, DIL = 32, 32, 8, 2
HALO = 16
NB = D // 128
EPS = 1e-5
NEG = -1e9
SCALE = DH ** -0.5
f32, bf16 = jnp.float32, jnp.bfloat16


def _ln(x):
    m = jnp.mean(x, axis=-1, keepdims=True)
    c = x - m
    v = jnp.mean(c * c, axis=-1, keepdims=True)
    return c * jax.lax.rsqrt(v + EPS)


def _dot(a, b):
    return jnp.dot(a, b, preferred_element_type=f32)


def make(TM=256, FC=512, NC=256, R=16, QC=512, LR=64, do_T=True, do_perm=True, vmem_mb=100, flags=None,
         order=None, no_ln=False, no_silu=False, parts='AUOD', t_slack=0, ln_in_down=False, alias=True, pin_ab=True, pin_xa=False):
    NT = S // TM
    NU = 2 * NT
    NFC = F // FC
    NNC = D // NC
    KC = 256

    def kernel(x0_ref, xn_ref, wqkv_h, wo_h, w1_h, w3_h, w2_h, o_ref,
               wqkv, wo, w1, w3, w2, tbuf, xs, kb, vb, comb, big, sems):
        _n = pl.program_id(0)
        z1 = (_n >> 20) if alias else 0
        hb = big.at[0]
        qb = big.at[1 + z1, :, pl.ds(0, D)]
        ab = big.at[1 + z1, :, pl.ds(D, D)] if pin_ab else comb.at[2]
        xa = big.at[1 + z1, :, pl.ds(2 * D, D)] if pin_xa else comb.at[0]
        xf = comb.at[1]
        n = pl.program_id(0)

        def qkv_copy(c):
            return pltpu.make_async_copy(wqkv_h.at[pl.ds(c * KC, KC)], wqkv.at[pl.ds(c * KC, KC)], sems.at[c])
        nq = D // KC
        wo_copy = pltpu.make_async_copy(wo_h, wo, sems.at[nq])
        w1_copy = pltpu.make_async_copy(w1_h, w1, sems.at[nq + 1])
        w3_copy = pltpu.make_async_copy(w3_h, w3, sems.at[nq + 2])
        w2_copy = pltpu.make_async_copy(w2_h, w2, sems.at[nq + 3])

        def permute_qkv(c):
            for m in range(3):
                blk = wqkv[pl.ds(c * KC, KC), pl.ds(m * D, D)]
                u = pltpu.bitcast(blk, jnp.uint32)
                tbuf[...] = u.T
                rows = [tbuf[pl.ds(d, H, stride=DH), :] for d in range(DH)]
                p = jnp.concatenate(rows, axis=0)
                wqkv[pl.ds(c * KC, KC), pl.ds(m * D, D)] = pltpu.bitcast(p.T, bf16)

        def permute_wo(j):
            cs = pl.ds(pl.multiple_of(j * 128, 128), 128)
            tbuf[...] = pltpu.bitcast(wo[:, cs].astype(f32), jnp.uint32)
            rows = [tbuf[pl.ds(d, H, stride=DH), :] for d in range(DH)]
            wo[:, cs] = pltpu.bitcast(jnp.concatenate(rows, axis=0), f32).astype(bf16)

        t = n % NT
        tp = jnp.maximum(n - 1, 0) % NT
        tn = (n + 1) % NT

        def ln_rows(dst, tile, r):
            r0 = r * LR if isinstance(r, int) else pl.multiple_of(r * LR, LR)
            rs = pl.ds(r0, LR)
            dst[rs, :] = _ln(xs[tile, rs, :]).astype(bf16)

        def a_dot(c):
            if 'A' not in parts: return
            res = _dot(xa[...], wqkv[:, pl.ds(c * QC, QC)])
            for jj in range(QC // 128):
                col = c * (QC // 128) + jj
                m, j = divmod(col, NB)
                piece = res[:, jj * 128:(jj + 1) * 128]
                if m == 0:
                    qb[:, pl.ds(j * 128, 128)] = piece.astype(bf16)
                elif m == 1:
                    kb[j, pl.ds(HALO, TM), :] = piece
                else:
                    vb[j, pl.ds(HALO, TM), :] = piece

        def halo_init():
            for j in range(NB):
                for buf in (kb, vb):
                    buf[j, pl.ds(0, HALO), :] = jnp.where(
                        t == 0, jnp.broadcast_to(buf[j, pl.ds(HALO, 1), :], (HALO, 128)), buf[j, pl.ds(0, HALO), :])

        def halo_carry():
            for j in range(NB):
                kb[j, pl.ds(0, HALO), :] = kb[j, pl.ds(TM, HALO), :]
                vb[j, pl.ds(0, HALO), :] = vb[j, pl.ds(TM, HALO), :]

        def t_piece(p):
            static = isinstance(p, int)
            r0 = p * R if static else pl.multiple_of(p * R, R)
            if not do_T:
                for j in range(NB):
                    ab[pl.ds(r0, R), pl.ds(j * 128, 128)] = (
                        qb[pl.ds(r0, R), pl.ds(j * 128, 128)].astype(f32) + kb[j, pl.ds(r0 + HALO, R), :] + vb[j, pl.ds(r0 + HALO, R), :]).astype(bf16)
                return
            lg = [None] * W
            for j in range(NB):
                q = qb[pl.ds(r0, R), pl.ds(j * 128, 128)].astype(f32)
                for w in range(W):
                    pr = q * kb[j, pl.ds(r0 + HALO - DIL * w, R), :]
                    lg[w] = pr if j == 0 else lg[w] + pr
            for w in range(W):
                a = lg[w]
                a = a + pltpu.roll(a, 64, 1)
                a = (a + pltpu.roll(a, 32, 1)) * SCALE
                if (not static) or r0 < DIL * w:
                    pos = t * TM + r0 + jax.lax.broadcasted_iota(jnp.int32, (R, 128), 0)
                    a = jnp.where(pos >= DIL * w, a, NEG)
                lg[w] = a
            mx = functools.reduce(jnp.maximum, lg)
            e = [jnp.exp(a - mx) for a in lg]
            inv = 1.0 / functools.reduce(lambda a, b: a + b, e)
            pw = [a * inv for a in e]
            for j in range(NB):
                acc = None
                for w in range(W):
                    pr = pw[w] * vb[j, pl.ds(r0 + HALO - DIL * w, R), :]
                    acc = pr if acc is None else acc + pr
                ab[pl.ds(r0, R), pl.ds(j * 128, 128)] = acc.astype(bf16)

        def o_dot(c):
            if 'O' not in parts: return
            cs = pl.ds(c * NC, NC)
            xs[t, :, cs] = xs[t, :, cs] + _dot(ab[...], wo[:, cs])

        def f_up(c):
            if 'U' not in parts: return
            cs = pl.ds(c * FC, FC)
            xv = xf[...]
            g = _dot(xv, w1[:, cs])
            u = _dot(xv, w3[:, cs])
            hb[:, cs] = ((g * u) if no_silu else (g * (1.0 / (1.0 + jnp.exp(-g))) * u)).astype(bf16)

        def f_down(c):
            if 'D' not in parts: return
            cs = pl.ds(c * NC, NC)
            y = xs[tp, :, cs] + _dot(hb[...], w2[:, cs])
            xs[tp, :, cs] = y
            o_ref[:, cs] = y.astype(o_ref.dtype)

        def stage_next_x():
            slot = jnp.where(n + 1 < NT, n + 1, NT)
            xs[slot] = xn_ref[...].astype(f32)

        NP = TM // R
        NQ = 3 * D // QC

        def loop(k, body):
            jax.lax.fori_loop(0, k, lambda i, c: (body(i), c)[1], 0)

        @pl.when(n == 0)
        def _prologue():
            for c in range(nq):
                qkv_copy(c).start()
            wo_copy.start()
            w1_copy.start()
            w3_copy.start()
            w2_copy.start()
            xs[0] = x0_ref[...].astype(f32)
            loop(TM // LR, lambda r: ln_rows(xa, 0, r))

            def perm(c):
                qkv_copy(c).wait()
                if do_perm:
                    permute_qkv(c)
            loop(nq, perm)

        @pl.when(n < NU)
        def _qkv():
            halo_carry()
            done = 0
            for c in range(NQ):
                a_dot(c)
                upto = ((TM // LR) * (c + 1)) // NQ
                for r in range(done, upto):
                    ln_rows(xf, tp, r)
                done = upto
            stage_next_x()

        @pl.when(n == NU)
        def _ln_only():
            loop(TM // LR, lambda r: ln_rows(xf, tp, r))

        @pl.when(n == 0)
        def _attn_only():
            halo_init()
            loop(NP, t_piece)
            loop(TM // LR, lambda r: ln_rows(xa, tn, r))
            wo_copy.wait()
            if do_perm:
                loop(NB, permute_wo)

        @pl.when(n == 1)
        def _wait_up():
            w1_copy.wait()
            w3_copy.wait()

        @pl.when(n > 0)
        def _up():
            halo_init()
            dt = dl = 0
            for c in range(NFC):
                f_up(c)
                upto = min(NP, (NP * (c + 1)) // (NFC - t_slack))
                for p in range(dt, upto):
                    t_piece(p)
                dt = upto
                if not ln_in_down:
                    upto = ((TM // LR) * (c + 1)) // NFC
                    for r in range(dl, upto):
                        ln_rows(xa, tn, r)
                    dl = upto

        @pl.when(n == 1)
        def _wait_down():
            w2_copy.wait()

        @pl.when(n > 0)
        def _down():
            dl = 0
            for c in range(NNC):
                f_down(c)
                if ln_in_down:
                    upto = ((TM // LR) * (c + 1)) // NNC
                    for r in range(dl, upto):
                        ln_rows(xa, tn, r)
                    dl = upto

        @pl.when(n < NU)
        def _oproj():
            for c in range(NNC):
                o_dot(c)

    any_spec = pl.BlockSpec(memory_space=pl.ANY)
    call = pl.pallas_call(
        kernel,
        grid=(NU + 1,),
        in_specs=[
            pl.BlockSpec((TM, D), lambda n: (0, 0)),
            pl.BlockSpec((TM, D), lambda n: (jnp.minimum(n + 1, NT - 1), 0)),
            any_spec, any_spec, any_spec, any_spec, any_spec,
        ],
        out_specs=pl.BlockSpec((TM, D), lambda n: (jnp.maximum(n - 1 - NT, 0), 0)),
        out_shape=jax.ShapeDtypeStruct((S, D), bf16),
        scratch_shapes=[
            pltpu.VMEM((D, 3 * D), bf16), pltpu.VMEM((D, D), bf16),
            pltpu.VMEM((D, F), bf16), pltpu.VMEM((D, F), bf16), pltpu.VMEM((F, D), bf16),
            pltpu.VMEM((D, 128), jnp.uint32),
            pltpu.VMEM((NT + 1, TM, D), f32),
            pltpu.VMEM((NB, TM + HALO, 128), f32),
            pltpu.VMEM((NB, TM + HALO, 128), f32),
            pltpu.VMEM((3, TM, D), bf16),
            pltpu.VMEM((2, TM, F), bf16),
            pltpu.SemaphoreType.DMA((D // KC + 4,)),
        ],
        compiler_params=pltpu.CompilerParams(
            dimension_semantics=("arbitrary",), vmem_limit_bytes=vmem_mb * 1024 * 1024, flags=flags),
    )

    @jax.jit
    def fn(A_x, A_wqkv, A_wo, B_x, B_w1, B_w3, B_w2):
        x = A_x.reshape(S, D)
        return call(x, x, A_wqkv, A_wo, B_w1, B_w3, B_w2).reshape(A_x.shape)
    return fn


_fn = make(TM=256,FC=256,QC=256,LR=16,alias=False,flags={'XLA_TPU_EVENLY_DISTRIBUTE_CRITICAL_NODES':True})


@jax.jit
def pallas_interleave_layers__sliding_local_dilated__glu_gated_swiglu__prompt_kernel(A_x, A_wqkv, A_wo, B_x, B_w1, B_w3, B_w2):
    return _fn(A_x, A_wqkv, A_wo, B_x, B_w1, B_w3, B_w2)
```

```python
import functools
import jax
import jax.numpy as jnp
from jax.experimental import pallas as pl
from jax.experimental.pallas import tpu as pltpu

S, D, F = 2048, 1024, 3584
H, DH, W, DIL = 32, 32, 8, 2
HALO = 16
NB = D // 128
EPS = 1e-5
NEG = -1e9
SCALE = DH ** -0.5
f32, bf16 = jnp.float32, jnp.bfloat16


def _ln(x):
    m = jnp.mean(x, axis=-1, keepdims=True)
    c = x - m
    v = jnp.mean(c * c, axis=-1, keepdims=True)
    return c * jax.lax.rsqrt(v + EPS)


def _dot(a, b):
    return jnp.dot(a, b, preferred_element_type=f32)


def _loop(k, body):
    jax.lax.fori_loop(0, k, lambda i, c: (body(i), c)[1], 0)


def make(TM=256, FC=512, NC=256, R=16, QC=256, LR=16, R0=32, LR0=128, KC=256, inflight=3, pitch=33, vmem_mb=100,
         flags=None, NL=2, t_slack=0, TU=16, late_norm=True, border='TAL', halo_first=True, stage_in='D', NCL=512, ln_in_down=False, stop=99):
    NT = S // TM
    NU = NL * NT
    FCS = list(FC) if isinstance(FC, (list, tuple)) else [FC] * (F // FC)
    assert sum(FCS) == F
    FOFF = [sum(FCS[:i]) for i in range(len(FCS) + 1)]
    NFC, NNC, NQ, NP, NLR = len(FCS), D // NC, 3 * D // QC, TM // R, TM // LR
    NKC = D // KC
    assert TM // R0 == NB

    def kernel(x_h, wqkv_h, wo_h, w1_h, w3_h, w2_h, o_ref,
               xin, wqkv, wo, w1, w3, w2, tbuf, xs, qkv, qkv0, xa, xf, ab, hb, sems):
        n = pl.program_id(0)
        t = n % NT
        tp = jnp.maximum(n - 1, 0) % NT
        cur, nxt = n % 2, (n + 1) % 2

        NPC = 3 * NKC

        def qkv_copy(i):
            blk = (pl.ds(pl.multiple_of((i // 3) * KC, KC), KC), pl.ds(pl.multiple_of((i % 3) * D, D), D))
            return pltpu.make_async_copy(wqkv_h.at[blk], wqkv.at[blk], sems.at[i])
        wo_copy = pltpu.make_async_copy(wo_h, wo, sems.at[NPC])
        w1_copy = pltpu.make_async_copy(w1_h, w1, sems.at[NPC + 1])
        w3_copy = pltpu.make_async_copy(w3_h, w3, sems.at[NPC + 2])
        w2_copy = pltpu.make_async_copy(w2_h, w2, sems.at[NPC + 3])

        def x_copy(i, r0, rows):
            return pltpu.make_async_copy(x_h.at[pl.ds(r0, rows)], xin.at[pl.ds(r0, rows)], sems.at[NPC + 4 + i])
        x_copies = [x_copy(0, 0, TM), x_copy(1, TM, 2 * TM), x_copy(3, 3 * TM, TM), x_copy(2, 4 * TM, S - 4 * TM)]

        def permute_qkv(src_r, dst_r, m):
            cs = pl.ds(pl.multiple_of(m * D, D), D)
            u = pltpu.bitcast(wqkv[pl.ds(pl.multiple_of(src_r, KC), KC), cs], jnp.uint32).T
            for h in range(H):
                tbuf[pl.ds(h * pitch, DH), :] = u[h * DH:(h + 1) * DH]
            p = jnp.concatenate([tbuf[pl.ds(d, H, stride=pitch), :] for d in range(DH)], axis=0)
            wqkv[pl.ds(pl.multiple_of(dst_r, KC), KC), cs] = pltpu.bitcast(p.T, bf16)

        def permute_wo(j):
            cs = pl.ds(pl.multiple_of(j * 128, 128), 128)
            for h in range(H):
                tbuf[pl.ds(h * pitch, DH), :] = pltpu.bitcast(wo[pl.ds(h * DH, DH), cs].astype(f32), jnp.uint32)
            for d in range(DH):
                wo[pl.ds(d * H, H), cs] = pltpu.bitcast(tbuf[pl.ds(d, H, stride=pitch), :], f32).astype(bf16)

        def row_slice(r, rows):
            return pl.ds(r * rows if isinstance(r, int) else pl.multiple_of(r * rows, rows), rows)

        def ln_rows(dst, tile, r, rows=LR):
            rs = row_slice(r, rows)
            dst[rs, :] = _ln(xs[tile, rs, :]).astype(bf16)

        def ln_input(tile, r, rows):
            rs = row_slice(r, rows)
            x = xin[row_slice(tile * (TM // rows) + r, rows), :].astype(f32)
            xs[tile, rs, :] = x
            xa[tile % 2, rs, :] = _ln(x).astype(bf16)

        def stage_rows(tile, r, rows=LR):
            xs[jnp.where(tile < NT, tile, NT), row_slice(r, rows), :] = xin[
                row_slice(jnp.minimum(tile, NT - 1) * (TM // rows) + r, rows), :].astype(f32)

        def a_dot(slot, c, cols):
            c0 = c * cols if isinstance(c, int) else pl.multiple_of(c * cols, 128)
            res = _dot(xa[slot], wqkv[pl.ds(0, D), pl.ds(c0, cols)])
            for jj in range(cols // 128):
                qkv[slot, c * (cols // 128) + jj, pl.ds(HALO, TM), :] = res[:, jj * 128:(jj + 1) * 128]

        def a_dot_partial(c, m):
            ks = pl.ds(pl.multiple_of(c * KC, KC), KC)
            res = _dot(xa[0, :, ks], wqkv[ks, pl.ds(pl.multiple_of(m * D, D), D)])
            for j in range(NB):
                dst = (m * NB + j, pl.ds(HALO, TM), slice(None))
                part = res[:, j * 128:(j + 1) * 128]
                qkv0[dst] = jnp.where(c == 0, part, qkv0[dst] + part)

        def halo_carry(dst, src):
            for j in range(NB, 3 * NB):
                dst[j, pl.ds(0, HALO), :] = src[j, pl.ds(TM, HALO), :]

        def halo_init(buf):
            for j in range(NB, 3 * NB):
                first = jnp.broadcast_to(buf[j, pl.ds(HALO, 1), :], (HALO, 128))
                buf[j, pl.ds(0, HALO), :] = jnp.where(t == 0, first, buf[j, pl.ds(0, HALO), :])

        def t_piece(buf, p, R=R):
            static = isinstance(p, int)
            r0 = p * R if static else pl.multiple_of(p * R, R)
            lg = [None] * W
            for j in range(NB):
                q = buf[j, pl.ds(r0 + HALO, R), :]
                for w in range(W):
                    pr = q * buf[NB + j, pl.ds(r0 + HALO - DIL * w, R), :]
                    lg[w] = pr if j == 0 else lg[w] + pr
            for w in range(W):
                a = lg[w]
                a = a + pltpu.roll(a, 64, 1)
                a = (a + pltpu.roll(a, 32, 1)) * SCALE
                if (not static) or r0 < DIL * w:
                    pos = t * TM + r0 + jax.lax.broadcasted_iota(jnp.int32, (R, 128), 0)
                    a = jnp.where(pos >= DIL * w, a, NEG)
                lg[w] = a
            mx = functools.reduce(jnp.maximum, lg)
            e = [jnp.exp(a - mx) for a in lg]
            inv = 1.0 / functools.reduce(lambda a, b: a + b, e)
            pw = e if late_norm else [a * inv for a in e]
            for j in range(NB):
                acc = None
                for w in range(W):
                    pr = pw[w] * buf[2 * NB + j, pl.ds(r0 + HALO - DIL * w, R), :]
                    acc = pr if acc is None else acc + pr
                ab[pl.ds(r0, R), pl.ds(j * 128, 128)] = (acc * inv if late_norm else acc).astype(bf16)

        def o_dot(c, cols):
            cs = pl.ds(c * cols if isinstance(c, int) else pl.multiple_of(c * cols, cols), cols)
            xs[t, :, cs] = xs[t, :, cs] + _dot(ab[...], wo[:, cs])

        def f_up(c):
            cs = pl.ds(FOFF[c], FCS[c])
            g = _dot(xf[...], w1[:, cs])
            u = _dot(xf[...], w3[:, cs])
            hb[:, cs] = (g * (1.0 / (1.0 + jnp.exp(-g))) * u).astype(bf16)

        def f_down(c):
            cs = pl.ds(c * NC, NC)
            y = xs[tp, :, cs] + _dot(hb[...], w2[:, cs])
            xs[tp, :, cs] = y
            o_ref[:, cs] = y.astype(o_ref.dtype)

        def spread(total, c, slots):
            return range(min(total, (total * c) // slots), min(total, (total * (c + 1)) // slots))

        @pl.when(n == 0)
        def _prologue():
            x_copies[0].start()
            qkv_copy(0).start()
            x_copies[0].wait()
            for i in range(1, inflight):
                qkv_copy(i).start()
            _loop(TM // LR0, lambda r: ln_input(0, r, LR0))

            def piece(i):
                @pl.when(i < NPC)
                def _():
                    qkv_copy(i).wait()

                @pl.when(i + inflight < NPC)
                def _():
                    qkv_copy(i + inflight).start()

                @pl.when(i + inflight == NPC)
                def _():
                    x_copies[1].start()

                @pl.when(i == NPC - 1)
                def _():
                    wo_copy.start()
                    x_copies[2].start()

                ip = jnp.maximum(i - 1, 0)
                a_dot_partial(ip // 3, ip % 3)
                permute_qkv(jnp.minimum(i // 3, NKC - 1) * KC, (i // 3) * KC, i % 3)
            _loop(NPC + 1, piece)

        @pl.when(n == 0)
        def _prologue2():
            halo_init(qkv0)
            halo_carry(qkv.at[1], qkv0)
            x_copies[1].wait()
            w1_copy.start()
            w3_copy.start()
            _loop(TM // LR0, lambda r: ln_input(1, r, LR0))

            def piece(p):
                for ch in border:
                    if ch == 'T': t_piece(qkv0, p, R0)
                    if ch == 'P': permute_wo(p)
                    if ch == 'L': ln_input(2, p, R0)
                    if ch == 'A': a_dot(1, p, 3 * D // NB)
            _loop(NB, piece)
            wo_copy.wait()
            x_copies[2].wait()
            _loop(NB, permute_wo)
            if stage_in == 'D': _loop(TM // LR0, lambda r: stage_rows(3, r, LR0))

        @pl.when(n == 1)
        def _wait_up():
            w1_copy.wait()
            w3_copy.wait()
            x_copies[3].start()
            w2_copy.start()

        @pl.when(n > 0)
        def _up():
            halo_init(qkv.at[cur])
            for c in range(NFC):
                f_up(c)
                for p in range(min(TU, TU * FOFF[c] // (F - t_slack)), min(TU, TU * FOFF[c + 1] // (F - t_slack))):
                    t_piece(qkv.at[cur], p)
                if not ln_in_down:
                    for r in range(min(NLR, NLR * FOFF[c] // (F - t_slack)), min(NLR, NLR * FOFF[c + 1] // (F - t_slack))):
                        ln_rows(xa.at[cur], (n + 2) % NT, r)

        @pl.when(n == 1)
        def _wait_down():
            w2_copy.wait()
            x_copies[3].wait()

        @pl.when(n > 0)
        def _down():
            for c in range(NNC):
                f_down(c)
                for p in spread(NP - TU, c, NNC):
                    t_piece(qkv.at[cur], TU + p)
                if stage_in == 'D':
                    for r in spread(NLR, c, NNC):
                        stage_rows(n + 3, r)
                if ln_in_down:
                    for r in spread(NLR, c, NNC):
                        ln_rows(xa.at[cur], (n + 2) % NT, r)

        @pl.when(n + 2 < NU)
        def _oproj_qkv():
            if halo_first: halo_carry(qkv.at[cur], qkv.at[nxt])
            for c in range(NNC):
                o_dot(c, NC)
            if not halo_first: halo_carry(qkv.at[cur], qkv.at[nxt])
            for c in range(NQ):
                a_dot(cur, c, QC)
                for r in spread(NLR, c, NQ):
                    ln_rows(xf, t, r)
                    if stage_in == 'A': stage_rows(n + 3, r)

        @pl.when(jnp.logical_and(n + 2 >= NU, n < NU))
        def _oproj():
            _loop(D // NCL, lambda c: o_dot(c, NCL))
            _loop(TM // LR0, lambda r: ln_rows(xf, t, r, LR0))

    any_spec = pl.BlockSpec(memory_space=pl.ANY)
    call = pl.pallas_call(
        kernel,
        grid=(min(NU + 1, stop),),
        in_specs=[
            any_spec, any_spec, any_spec, any_spec, any_spec, any_spec,
        ],
        out_specs=pl.BlockSpec((TM, D), lambda n: (jnp.maximum(n - 1 - (NU - NT), 0), 0)),
        out_shape=jax.ShapeDtypeStruct((S, D), bf16),
        scratch_shapes=[
            pltpu.VMEM((S, D), bf16),
            pltpu.VMEM((D + KC, 3 * D), bf16), pltpu.VMEM((D, D), bf16),
            pltpu.VMEM((D, F), bf16), pltpu.VMEM((D, F), bf16), pltpu.VMEM((F, D), bf16),
            pltpu.VMEM((H * 40, 128), jnp.uint32),
            pltpu.VMEM((NT + 1, TM, D), f32),
            pltpu.VMEM((2, 3 * NB, TM + HALO, 128), f32),
            pltpu.VMEM((3 * NB, TM + HALO, 128), f32),
            pltpu.VMEM((2, TM, D), bf16), pltpu.VMEM((TM, D), bf16), pltpu.VMEM((TM, D), bf16),
            pltpu.VMEM((TM, F), bf16),
            pltpu.SemaphoreType.DMA((3 * NKC + 8,)),
        ],
        compiler_params=pltpu.CompilerParams(
            dimension_semantics=("arbitrary",), vmem_limit_bytes=vmem_mb * 1024 * 1024, flags=flags),
    )

    def fn(A_x, A_wqkv, A_wo, B_x, B_w1, B_w3, B_w2):
        x = A_x.reshape(S, D)
        return call(x, A_wqkv, A_wo, B_w1, B_w3, B_w2).reshape(A_x.shape)
    return jax.jit(fn)


_fn = make(flags={'XLA_TPU_EVENLY_DISTRIBUTE_CRITICAL_NODES':True})


@jax.jit
def pallas_interleave_layers__sliding_local_dilated__glu_gated_swiglu__prompt_kernel(A_x, A_wqkv, A_wo, B_x, B_w1, B_w3, B_w2):
    return _fn(A_x, A_wqkv, A_wo, B_x, B_w1, B_w3, B_w2)
```

```python
import functools
import jax
import jax.numpy as jnp
from jax.experimental import pallas as pl
from jax.experimental.pallas import tpu as pltpu

S, D, F = 2048, 1024, 3584
H, DH, W, DIL = 32, 32, 8, 2
HALO = 16
NB = D // 128
EPS = 1e-5
NEG = -1e9
SCALE = DH ** -0.5
f32, bf16 = jnp.float32, jnp.bfloat16


def _ln(x):
    m = jnp.mean(x, axis=-1, keepdims=True)
    c = x - m
    v = jnp.mean(c * c, axis=-1, keepdims=True)
    return c * jax.lax.rsqrt(v + EPS)


def _dot(a, b):
    return jnp.dot(a, b, preferred_element_type=f32)


def _loop(k, body):
    jax.lax.fori_loop(0, k, lambda i, c: (body(i), c)[1], 0)


def make(TM=256, FC=512, NC=512, R=16, QC=512, LR=16, R0=32, LR0=128, KC=256, inflight=3, pitch=33, vmem_mb=100,
         flags=None, NL=2, t_slack=0, TU=16, late_norm=True, PU=1, OS=1, split_ud=True, silu='tanh', border='TAL', halo_first=True, stage_in='D', NCL=512, ln_in_down=False, stop=99):
    NT = S // TM
    NU = NL * NT
    FCS = list(FC) if isinstance(FC, (list, tuple)) else [FC] * (F // FC)
    assert sum(FCS) == F
    FOFF = [sum(FCS[:i]) for i in range(len(FCS) + 1)]
    NFC, NNC, NQ, NP, NLR = len(FCS), D // NC, 3 * D // QC, TM // R, TM // LR
    NKC = D // KC
    NBI = TM // R0

    def kernel(x_h, wqkv_h, wo_h, w1_h, w3_h, w2_h, o_h,
               xin, wqkv, wo, w1, w3, w2, tbuf, xs, qkv, qkv0, xa, xf, ab, hb, ob, sems):
        NPC = 3 * NKC

        def qkv_copy(i):
            blk = (pl.ds(pl.multiple_of((i // 3) * KC, KC), KC), pl.ds(pl.multiple_of((i % 3) * D, D), D))
            return pltpu.make_async_copy(wqkv_h.at[blk], wqkv.at[blk], sems.at[i])
        wo_copy = pltpu.make_async_copy(wo_h, wo, sems.at[NPC])
        w1_copy = pltpu.make_async_copy(w1_h, w1, sems.at[NPC + 1])
        w3_copy = pltpu.make_async_copy(w3_h, w3, sems.at[NPC + 2])
        w2_copy = pltpu.make_async_copy(w2_h, w2, sems.at[NPC + 3])

        def x_copy(i, r0, rows):
            return pltpu.make_async_copy(x_h.at[pl.ds(r0, rows)], xin.at[pl.ds(r0, rows)], sems.at[NPC + 4 + i])
        x_copies = [x_copy(0, 0, TM), x_copy(1, TM, 3 * TM), x_copy(2, 4 * TM, S - 4 * TM)]

        def permute_qkv(src_r, dst_r, m):
            al = lambda v, k: v if isinstance(v, int) else pl.multiple_of(v, k)
            cs = pl.ds(al(m * D, D), D)
            u = pltpu.bitcast(wqkv[pl.ds(al(src_r, KC), KC), cs], jnp.uint32).T
            for h in range(H):
                tbuf[pl.ds(h * pitch, DH), :] = u[h * DH:(h + 1) * DH]
            p = jnp.concatenate([tbuf[pl.ds(d, H, stride=pitch), :] for d in range(DH)], axis=0)
            wqkv[pl.ds(al(dst_r, KC), KC), cs] = pltpu.bitcast(p.T, bf16)

        def permute_wo(j):
            cs = pl.ds(pl.multiple_of(j * 128, 128), 128)
            for h in range(H):
                tbuf[pl.ds(h * pitch, DH), :] = pltpu.bitcast(wo[pl.ds(h * DH, DH), cs].astype(f32), jnp.uint32)
            for d in range(DH):
                wo[pl.ds(d * H, H), cs] = pltpu.bitcast(tbuf[pl.ds(d, H, stride=pitch), :], f32).astype(bf16)

        def row_slice(r, rows):
            return pl.ds(r * rows if isinstance(r, int) else pl.multiple_of(r * rows, rows), rows)

        def ln_rows(dst, tile, r, rows=LR):
            rs = row_slice(r, rows)
            dst[rs, :] = _ln(xs[tile, rs, :]).astype(bf16)

        def resid(u, r, rows, cs=slice(None)):
            x0 = xin[row_slice((u % NT) * (TM // rows) + r, rows), cs].astype(f32)
            if isinstance(u, int):
                assert u < NT
                return x0
            return jnp.where(u < NT, x0, xs[u % NT, row_slice(r, rows), cs])

        def ln_attn(u, r, rows=LR):
            xa[u % 2, row_slice(r, rows), :] = _ln(resid(u, r, rows)).astype(bf16)

        def a_dot(slot, c, cols):
            c0 = c * cols if isinstance(c, int) else pl.multiple_of(c * cols, 128)
            res = _dot(xa[slot], wqkv[pl.ds(0, D), pl.ds(c0, cols)])
            for jj in range(cols // 128):
                qkv[slot, c * (cols // 128) + jj, pl.ds(HALO, TM), :] = res[:, jj * 128:(jj + 1) * 128]

        def a_dot_partial(c, m):
            ks = pl.ds(pl.multiple_of(c * KC, KC), KC)
            res = _dot(xa[0, :, ks], wqkv[ks, pl.ds(pl.multiple_of(m * D, D), D)])
            for j in range(NB):
                dst = (m * NB + j, pl.ds(HALO, TM), slice(None))
                part = res[:, j * 128:(j + 1) * 128]
                qkv0[dst] = jnp.where(c == 0, part, qkv0[dst] + part)

        def halo_carry(dst, src):
            for j in range(NB, 3 * NB):
                dst[j, pl.ds(0, HALO), :] = src[j, pl.ds(TM, HALO), :]

        def halo_init(buf, t):
            for j in range(NB, 3 * NB):
                first = jnp.broadcast_to(buf[j, pl.ds(HALO, 1), :], (HALO, 128))
                buf[j, pl.ds(0, HALO), :] = jnp.where(t == 0, first, buf[j, pl.ds(0, HALO), :])

        def t_piece(buf, t, p, R=R):
            static = isinstance(p, int)
            r0 = p * R if static else pl.multiple_of(p * R, R)
            lg = [None] * W
            for j in range(NB):
                q = buf[j, pl.ds(r0 + HALO, R), :]
                for w in range(W):
                    pr = q * buf[NB + j, pl.ds(r0 + HALO - DIL * w, R), :]
                    lg[w] = pr if j == 0 else lg[w] + pr
            for w in range(W):
                a = lg[w]
                a = a + pltpu.roll(a, 64, 1)
                a = (a + pltpu.roll(a, 32, 1)) * SCALE
                if (not static) or r0 < DIL * w:
                    pos = t * TM + r0 + jax.lax.broadcasted_iota(jnp.int32, (R, 128), 0)
                    a = jnp.where(pos >= DIL * w, a, NEG)
                lg[w] = a
            mx = functools.reduce(jnp.maximum, lg)
            e = [jnp.exp(a - mx) for a in lg]
            inv = 1.0 / functools.reduce(lambda a, b: a + b, e)
            pw = e if late_norm else [a * inv for a in e]
            for j in range(NB):
                acc = None
                for w in range(W):
                    pr = pw[w] * buf[2 * NB + j, pl.ds(r0 + HALO - DIL * w, R), :]
                    acc = pr if acc is None else acc + pr
                ab[pl.ds(r0, R), pl.ds(j * 128, 128)] = (acc * inv if late_norm else acc).astype(bf16)

        def o_dot(u, c, cols, r=0, rows=TM):
            cs = pl.ds(c * cols if isinstance(c, int) else pl.multiple_of(c * cols, cols), cols)
            rs = row_slice(r, rows)
            xs[u % NT, rs, cs] = resid(u, r, rows, cs) + _dot(ab[rs, :], wo[:, cs])

        def f_up(c):
            cs = pl.ds(FOFF[c], FCS[c])
            g = _dot(xf[...], w1[:, cs])
            u = _dot(xf[...], w3[:, cs])
            if silu == 'tanh':
                hg = 0.5 * g
                act = hg * jnp.tanh(hg) + hg
            else:
                act = g * (1.0 / (1.0 + jnp.exp(-g)))
            hb[:, cs] = (act * u).astype(bf16)

        def f_down(tp, c):
            cs = pl.ds(c * NC, NC)
            y = xs[tp, :, cs] + _dot(hb[...], w2[:, cs])
            xs[tp, :, cs] = y
            ob[:, cs] = y.astype(ob.dtype)

        def spread(total, c, slots):
            return range(min(total, (total * c) // slots), min(total, (total * (c + 1)) // slots))

        with jax.named_scope('_prologue'):
            x_copies[0].start()
            qkv_copy(0).start()
            x_copies[0].wait()
            for i in range(1, inflight):
                qkv_copy(i).start()
            _loop(TM // LR0, lambda r: ln_attn(0, r, LR0))

            def dma(i):
                @pl.when(i < NPC)
                def _():
                    qkv_copy(i).wait()

                @pl.when(i + inflight < NPC)
                def _():
                    qkv_copy(i + inflight).start()

                @pl.when(i + inflight == NPC)
                def _():
                    x_copies[1].start()

                @pl.when(i == NPC - 1)
                def _():
                    wo_copy.start()

            def piece(k):
                for i in range(PU):
                    dma(k * PU + i + (PU > 1))
                for i in range(PU):
                    i = k * PU + i + (PU > 1)
                    ip = jnp.maximum(i - 1, 0)
                    a_dot_partial(ip // 3, ip % 3)
                    permute_qkv(jnp.minimum(i // 3, NKC - 1) * KC, (i // 3) * KC, i % 3)
            if PU > 1:
                dma(jnp.int32(0))
                permute_qkv(0, 0, 0)
                _loop(NPC // PU, piece)
            else:
                _loop(NPC + 1, piece)

        with jax.named_scope('_prologue2'):
            halo_init(qkv0, 0)
            halo_carry(qkv.at[1], qkv0)
            x_copies[1].wait()
            w1_copy.start()
            w3_copy.start()
            _loop(TM // LR0, lambda r: ln_attn(1, r, LR0))

            def piece(p):
                for ch in border:
                    if ch == 'T': t_piece(qkv0, 0, p, R0)
                    if ch == 'P': permute_wo(p)
                    if ch == 'L': ln_attn(2, p, R0)
                    if ch == 'A': a_dot(1, p, 3 * D // NBI)
            _loop(NBI, piece)
            wo_copy.wait()
            _loop(NB, permute_wo)

        def out_copy(tile):
            return pltpu.make_async_copy(ob, o_h.at[row_slice(tile, TM)], sems.at[NPC + 8])

        def step(u):
            t, t1 = u % NT, (u + 1) % NT
            s0, s1 = u % 2, (u + 1) % 2

            @pl.when(u + 2 < NU)
            def _oproj_qkv():
                halo_carry(qkv.at[s0], qkv.at[s1])
                for h in range(OS):
                    for c in range(NNC):
                        o_dot(u, c, NC, h, TM // OS)
                    if h < OS - 1:
                        for r in spread(NLR, h, OS):
                            ln_rows(xf, t, r)
                rest = list(spread(NLR, OS - 1, OS))
                for c in range(NQ):
                    a_dot(s0, c, QC)
                    for i in spread(len(rest), c, NQ):
                        ln_rows(xf, t, rest[i])

            @pl.when(u + 2 >= NU)
            def _oproj():
                _loop(D // NCL, lambda c: o_dot(u, c, NCL))
                _loop(TM // LR0, lambda r: ln_rows(xf, t, r, LR0))

            @pl.when(u == 0)
            def _wait_up():
                w1_copy.wait()
                w3_copy.wait()
                x_copies[2].start()
                w2_copy.start()
                if not split_ud: w2_copy.wait()

            @pl.when(u == 1)
            def _wait_x():
                x_copies[2].wait()

            @pl.when(u > NU - NT)
            def _wait_out():
                out_copy(t).wait()

            halo_init(qkv.at[s1], t1)
            for c in range(NFC):
                f_up(c)
                for p in range(NP * FOFF[c] // F, NP * FOFF[c + 1] // F):
                    t_piece(qkv.at[s1], t1, p)
                for r in range(NLR * FOFF[c] // F, NLR * FOFF[c + 1] // F):
                    ln_attn(u + 3, r)

            if split_ud:
                @pl.when(u == 0)
                def _wait_down():
                    w2_copy.wait()

            for c in range(NNC):
                f_down(t, c)

            @pl.when(u >= NU - NT)
            def _start_out():
                out_copy(t).start()

        _loop(NU, step)
        out_copy(NT - 1).wait()

    any_spec = pl.BlockSpec(memory_space=pl.ANY)
    call = pl.pallas_call(
        kernel,
        in_specs=[
            any_spec, any_spec, any_spec, any_spec, any_spec, any_spec,
        ],
        out_specs=any_spec,
        out_shape=jax.ShapeDtypeStruct((S, D), bf16),
        scratch_shapes=[
            pltpu.VMEM((S, D), bf16),
            pltpu.VMEM((D + KC, 3 * D), bf16), pltpu.VMEM((D, D), bf16),
            pltpu.VMEM((D, F), bf16), pltpu.VMEM((D, F), bf16), pltpu.VMEM((F, D), bf16),
            pltpu.VMEM((H * 40, 128), jnp.uint32),
            pltpu.VMEM((NT, TM, D), f32),
            pltpu.VMEM((2, 3 * NB, TM + HALO, 128), f32),
            pltpu.VMEM((3 * NB, TM + HALO, 128), f32),
            pltpu.VMEM((2, TM, D), bf16), pltpu.VMEM((TM, D), bf16), pltpu.VMEM((TM, D), bf16),
            pltpu.VMEM((TM, F), bf16), pltpu.VMEM((TM, D), bf16),
            pltpu.SemaphoreType.DMA((3 * NKC + 9,)),
        ],
        compiler_params=pltpu.CompilerParams(
            vmem_limit_bytes=vmem_mb * 1024 * 1024, flags=flags),
    )

    def fn(A_x, A_wqkv, A_wo, B_x, B_w1, B_w3, B_w2):
        x = A_x.reshape(S, D)
        return call(x, A_wqkv, A_wo, B_w1, B_w3, B_w2).reshape(A_x.shape)
    return jax.jit(fn)


_fn = make(R0=64, NCL=1024, flags={'XLA_TPU_EVENLY_DISTRIBUTE_CRITICAL_NODES': True})


@jax.jit
def pallas_interleave_layers__sliding_local_dilated__glu_gated_swiglu__prompt_kernel(A_x, A_wqkv, A_wo, B_x, B_w1, B_w3, B_w2):
    return _fn(A_x, A_wqkv, A_wo, B_x, B_w1, B_w3, B_w2)
```

```python
import functools
import jax
import jax.numpy as jnp
from jax.experimental import pallas as pl
from jax.experimental.pallas import tpu as pltpu

S, D, F = 2048, 1024, 3584
H, DH, W, DIL = 32, 32, 8, 2
HALO = 16
NB = D // 128
EPS = 1e-5
NEG = -1e9
SCALE = DH ** -0.5
f32, bf16 = jnp.float32, jnp.bfloat16
DHALF, FH = D // 2, F // 2


def _ln(x):
    m = jnp.mean(x, axis=-1, keepdims=True)
    c = x - m
    v = jnp.mean(c * c, axis=-1, keepdims=True)
    return c * jax.lax.rsqrt(v + EPS)


def _dot(a, b):
    return jnp.dot(a, b, preferred_element_type=f32)


def _loop(k, body):
    jax.lax.fori_loop(0, k, lambda i, c: (body(i), c)[1], 0)


def _lhs_terms(a11, a12, a21, a22):
    return (a11 + a22, a21 + a22, a11, a22, a11 + a12, a21 - a11, a12 - a22)


def _rhs_terms(b11, b12, b21, b22):
    return (b11 + b22, b11, b12 - b22, b21 - b11, b22, b11 + b12, b21 + b22)


def _strassen(prod):
    m0, m1, m2, m3, m4 = (prod(i) for i in range(5))
    c12, c21 = m2 + m4, m1 + m3
    c22 = (m0 - m1) + m2 + prod(5)
    c11 = (m0 + m3) - m4 + prod(6)
    return c11, c12, c21, c22


def make(TM=256, FC=(512, 512, 512, 256), DC=256, WR=64, NC=256, R=16, QC=256, LR=16, R0=64, LR0=128, KC=256, inflight=3, pitch=33, vmem_mb=110,
         flags=None, NL=2, t_slack=0, late_norm=True, t_first=False, ln_pos='U', wout=False, ufirst=True, TU=8, tree=False, PU=1, OS=1, split_ud=True, silu='tanh', border='TAL', halo_first=True, stage_in='D', NCL=512, ln_in_down=False, stop=99):
    NT = S // TM
    NU = NL * NT
    FCS = list(FC) if isinstance(FC, (list, tuple)) else [FC] * (FH // FC)
    assert sum(FCS) == FH
    FOFF = [sum(FCS[:i]) for i in range(len(FCS) + 1)]
    NFC, NNC, NQ, NP, NLR = len(FCS), DHALF // NC, 3 * DHALF // QC, TM // 2 // R, TM // 2 // LR
    NKC = D // KC
    TH = TM // 2
    NBI = TM // R0

    def kernel(x_h, wqkv_h, wo_h, w1_h, w3_h, w2_h, o_h,
               xin, wqkv, wo, wqkv7, wo7, w1, w3, w2, tbuf, xs, qkv, qkv0, x0, xa, xf, ab, hb, ob, sems):
        NPC = 3 * NKC

        def qkv_copy(i):
            blk = (pl.ds(pl.multiple_of((i // 3) * KC, KC), KC), pl.ds(pl.multiple_of((i % 3) * D, D), D))
            return pltpu.make_async_copy(wqkv_h.at[blk], wqkv.at[blk], sems.at[i])
        wo_copy = pltpu.make_async_copy(wo_h, wo, sems.at[NPC])

        def block_copies(w_h, w, sem0):
            kh, nh = w.shape[1:]
            return [pltpu.make_async_copy(w_h.at[pl.ds(i * kh, kh), pl.ds(j * nh, nh)], w.at[1 + 2 * i + j],
                                          sems.at[sem0 + 2 * i + j]) for i in range(2) for j in range(2)]
        w1_copies = block_copies(w1_h, w1, NPC + 9)
        w3_copies = block_copies(w3_h, w3, NPC + 13)
        w2_copies = block_copies(w2_h, w2, NPC + 17)

        def rhs_terms(w, rows):
            def body(r):
                rs = row_slice(r, rows)
                b11, b12, b21, b22 = (w[i, rs, :].astype(f32) for i in (1, 2, 3, 4))
                for i, term in enumerate(_rhs_terms(b11, b12, b21, b22)):
                    if i not in (1, 4):
                        w[i, rs, :] = term.astype(bf16)
            _loop(w.shape[1] // rows, body)

        def proj_terms(dst, src, rows):
            def body(r):
                top, bot = row_slice(r, rows), row_slice(DHALF // rows + r, rows)
                for m in range(src.shape[1] // D):
                    left, right = pl.ds(m * D, DHALF), pl.ds(m * D + DHALF, DHALF)
                    quads = (src[rs, cs].astype(f32) for rs in (top, bot) for cs in (left, right))
                    for i, term in enumerate(_rhs_terms(*quads)):
                        dst[i, top, pl.ds(m * DHALF, DHALF)] = term.astype(bf16)
            _loop(DHALF // rows, body)

        def x_copy(i, r0, rows):
            return pltpu.make_async_copy(x_h.at[pl.ds(r0, rows)], xin.at[pl.ds(r0, rows)], sems.at[NPC + 4 + i])
        x_copies = [x_copy(0, 0, TM), x_copy(1, TM, 3 * TM), x_copy(2, 4 * TM, S - 4 * TM)]

        def permute_qkv(src_r, dst_r, m):
            al = lambda v, k: v if isinstance(v, int) else pl.multiple_of(v, k)
            cs = pl.ds(al(m * D, D), D)
            u = pltpu.bitcast(wqkv[pl.ds(al(src_r, KC), KC), cs], jnp.uint32).T
            for h in range(H):
                tbuf[pl.ds(h * pitch, DH), :] = u[h * DH:(h + 1) * DH]
            p = jnp.concatenate([tbuf[pl.ds(d, H, stride=pitch), :] for d in range(DH)], axis=0)
            wqkv[pl.ds(al(dst_r, KC), KC), cs] = pltpu.bitcast(p.T, bf16)

        def permute_wo(j):
            cs = pl.ds(pl.multiple_of(j * 128, 128), 128)
            for h in range(H):
                tbuf[pl.ds(h * pitch, DH), :] = pltpu.bitcast(wo[pl.ds(h * DH, DH), cs].astype(f32), jnp.uint32)
            for d in range(DH):
                wo[pl.ds(d * H, H), cs] = pltpu.bitcast(tbuf[pl.ds(d, H, stride=pitch), :], f32).astype(bf16)

        def row_slice(r, rows):
            return pl.ds(r * rows if isinstance(r, int) else pl.multiple_of(r * rows, rows), rows)

        def store_lhs(dst, rs, top, bot):
            terms = _lhs_terms(top[:, :DHALF], top[:, DHALF:], bot[:, :DHALF], bot[:, DHALF:])
            for i, term in enumerate(terms):
                dst[i, rs, :] = term.astype(bf16)

        def ln_ffn(tile, r, rows=LR):
            top, bot = (_ln(xs[tile, row_slice(k, rows), :]) for k in (r, TH // rows + r))
            store_lhs(xf, row_slice(r, rows), top, bot)

        def resid(u, r, rows, cs=slice(None)):
            x0 = xin[row_slice((u % NT) * (TM // rows) + r, rows), cs].astype(f32)
            if isinstance(u, int):
                assert u < NT
                return x0
            return jnp.where(u < NT, x0, xs[u % NT, row_slice(r, rows), cs])

        def ln_attn(u, r, rows=LR):
            top, bot = (_ln(resid(u, k, rows)) for k in (r, TH // rows + r))
            store_lhs(xa.at[u % 2], row_slice(r, rows), top, bot)

        def ln_first(r, rows):
            x0[row_slice(r, rows), :] = _ln(resid(0, r, rows)).astype(bf16)

        def a_dot(slot, c, cols):
            c0 = c * cols if isinstance(c, int) else pl.multiple_of(c * cols, 128)
            out = _strassen(lambda i: _dot(xa[slot, i], wqkv7[i, :, pl.ds(c0, cols)]))
            for jj in range(cols // 128):
                k = c * (cols // 128) + jj
                slab = (k // (NB // 2)) * NB + k % (NB // 2)
                for i, o in enumerate(out):
                    qkv[slot, slab + (i % 2) * (NB // 2), pl.ds(HALO + (i // 2) * TH, TH), :] = o[:, jj * 128:(jj + 1) * 128]

        def a_dot_partial(c, m):
            ks = pl.ds(pl.multiple_of(c * KC, KC), KC)
            res = _dot(x0[:, ks], wqkv[ks, pl.ds(pl.multiple_of(m * D, D), D)])
            for j in range(NB):
                dst = (m * NB + j, pl.ds(HALO, TM), slice(None))
                part = res[:, j * 128:(j + 1) * 128]
                qkv0[dst] = jnp.where(c == 0, part, qkv0[dst] + part)

        def halo_carry(dst, src):
            for j in range(NB, 3 * NB):
                dst[j, pl.ds(0, HALO), :] = src[j, pl.ds(TM, HALO), :]

        def halo_init(buf, t):
            for j in range(NB, 3 * NB):
                first = jnp.broadcast_to(buf[j, pl.ds(HALO, 1), :], (HALO, 128))
                buf[j, pl.ds(0, HALO), :] = jnp.where(t == 0, first, buf[j, pl.ds(0, HALO), :])

        def attend(buf, t, p, R):
            static = isinstance(p, int)
            r0 = p * R if static else pl.multiple_of(p * R, R)
            lg = [None] * W
            q = [buf[j, pl.ds(r0 + HALO, R), :] for j in range(NB)]
            for j, w in ([(j, w) for w in range(W) for j in range(NB)] if wout else [(j, w) for j in range(NB) for w in range(W)]):
                pr = q[j] * buf[NB + j, pl.ds(r0 + HALO - DIL * w, R), :]
                lg[w] = pr if j == 0 else lg[w] + pr
            for w in range(W):
                a = lg[w]
                a = a + pltpu.roll(a, 64, 1)
                a = (a + pltpu.roll(a, 32, 1)) * SCALE
                if (not static) or r0 < DIL * w:
                    pos = t * TM + r0 + jax.lax.broadcasted_iota(jnp.int32, (R, 128), 0)
                    a = jnp.where(pos >= DIL * w, a, NEG)
                lg[w] = a
            mx = functools.reduce(jnp.maximum, lg)
            e = [jnp.exp(a - mx) for a in lg]
            inv = 1.0 / functools.reduce(lambda a, b: a + b, e)
            pw = e if late_norm else [a * inv for a in e]
            out = []
            for j in range(NB):
                acc = None
                for w in range(W):
                    pr = pw[w] * buf[2 * NB + j, pl.ds(r0 + HALO - DIL * w, R), :]
                    acc = pr if acc is None else acc + pr
                out.append(acc * inv if late_norm else acc)
            return jnp.concatenate(out, axis=1)

        def t_piece(buf, t, p, R=R):
            store_lhs(ab, row_slice(p, R), attend(buf, t, p, R), attend(buf, t, TH // R + p, R))

        def o_dot(u, c, cols):
            c0 = c * cols if isinstance(c, int) else pl.multiple_of(c * cols, cols)
            out = _strassen(lambda i: _dot(ab[i], wo7[i, :, pl.ds(c0, cols)]))
            for i, o in enumerate(out):
                cs = pl.ds((i % 2) * DHALF + c0, cols)
                xs[u % NT, row_slice(i // 2, TH), cs] = resid(u, i // 2, TH, cs) + o

        def f_up(c):
            cs = pl.ds(FOFF[c], FCS[c])
            up = _strassen(lambda i: _dot(xf[i], w3[i, :, cs]))
            gate = _strassen(lambda i: _dot(xf[i], w1[i, :, cs]))
            h = []
            for g, u in zip(gate, up):
                hg = 0.5 * g
                h.append((hg * jnp.tanh(hg) + hg) * u)
            for i, term in enumerate(_lhs_terms(*h)):
                hb[i, :, cs] = term.astype(bf16)

        def f_down(tp, c):
            out = _strassen(lambda i: _dot(hb[i], w2[i, :, pl.ds(c * DC, DC)]))
            for i, o in enumerate(out):
                rs, cs = pl.ds((i // 2) * TH, TH), pl.ds((i % 2) * DHALF + c * DC, DC)
                y = xs[tp, rs, cs] + o
                xs[tp, rs, cs] = y
                ob[rs, cs] = y.astype(ob.dtype)

        def spread(total, c, slots):
            return range(min(total, (total * c) // slots), min(total, (total * (c + 1)) // slots))

        with jax.named_scope('_prologue'):
            x_copies[0].start()
            qkv_copy(0).start()
            x_copies[0].wait()
            for i in range(1, inflight):
                qkv_copy(i).start()
            _loop(TM // LR0, lambda r: ln_first(r, LR0))

            def dma(i):
                @pl.when(i < NPC)
                def _():
                    qkv_copy(i).wait()

                @pl.when(i + inflight < NPC)
                def _():
                    qkv_copy(i + inflight).start()

                @pl.when(i + inflight == NPC)
                def _():
                    x_copies[1].start()

                @pl.when(i == NPC - 1)
                def _():
                    wo_copy.start()

            def piece(k):
                for i in range(PU):
                    dma(k * PU + i + (PU > 1))
                for i in range(PU):
                    i = k * PU + i + (PU > 1)
                    ip = jnp.maximum(i - 1, 0)
                    a_dot_partial(ip // 3, ip % 3)
                    permute_qkv(jnp.minimum(i // 3, NKC - 1) * KC, (i // 3) * KC, i % 3)
            if PU > 1:
                dma(jnp.int32(0))
                permute_qkv(0, 0, 0)
                _loop(NPC // PU, piece)
            else:
                _loop(NPC + 1, piece)

        with jax.named_scope('_prologue2'):
            halo_init(qkv0, 0)
            halo_carry(qkv.at[1], qkv0)
            x_copies[1].wait()
            for cp in w3_copies + w1_copies:
                cp.start()
            _loop(TM // LR0, lambda r: ln_attn(1, r, LR0 // 2))
            proj_terms(wqkv7, wqkv, WR // 2)

            def piece(p):
                for ch in border:
                    if ch == 'T': t_piece(qkv0, 0, p, R0 // 2)
                    if ch == 'P': permute_wo(p)
                    if ch == 'L': ln_attn(2, p, R0 // 2)
                    if ch == 'A': a_dot(1, p, 3 * DHALF // NBI)
            _loop(NBI, piece)
            wo_copy.wait()
            _loop(NB, permute_wo)
            proj_terms(wo7, wo, 2 * WR)

        def out_copy(tile):
            return pltpu.make_async_copy(ob, o_h.at[row_slice(tile, TM)], sems.at[NPC + 8])

        def step(u):
            t, t1 = u % NT, (u + 1) % NT
            s0, s1 = u % 2, (u + 1) % 2

            @pl.when(u + 2 < NU)
            def _oproj_qkv():
                halo_carry(qkv.at[s0], qkv.at[s1])
                for c in range(NNC):
                    o_dot(u, c, NC)
                for c in range(NQ):
                    a_dot(s0, c, QC)
                    for r in spread(NLR, c, NQ):
                        ln_ffn(t, r)

            @pl.when(u + 2 >= NU)
            def _oproj():
                for c in range(DHALF // NCL):
                    o_dot(u, c, NCL)
                _loop(TM // LR0, lambda r: ln_ffn(t, r, LR0 // 2))

            @pl.when(u == 0)
            def _wait_up():
                for cp in w3_copies:
                    cp.wait()
                rhs_terms(w3, WR // 2)
                for cp in w1_copies:
                    cp.wait()
                x_copies[2].start()
                for cp in w2_copies:
                    cp.start()
                rhs_terms(w1, WR // 2)

            @pl.when(u == 1)
            def _wait_x():
                x_copies[2].wait()

            @pl.when(u > NU - NT)
            def _wait_out():
                out_copy(t).wait()

            halo_init(qkv.at[s1], t1)
            for c in range(NFC):
                if not t_first: f_up(c)
                for p in range(TU * FOFF[c] // FH, TU * FOFF[c + 1] // FH):
                    t_piece(qkv.at[s1], t1, p)
                if ln_pos == 'U':
                    for r in range(NLR * FOFF[c] // FH, NLR * FOFF[c + 1] // FH):
                        ln_attn(u + 3, r)
                if t_first: f_up(c)

            if split_ud:
                @pl.when(u == 0)
                def _wait_down():
                    for cp in w2_copies:
                        cp.wait()
                    rhs_terms(w2, 2 * WR)

            for c in range(DHALF // DC):
                f_down(t, c)
                for p in spread(NP - TU, c, DHALF // DC):
                    t_piece(qkv.at[s1], t1, TU + p)
                if ln_pos == 'D':
                    for r in spread(NLR, c, DHALF // DC):
                        ln_attn(u + 3, r)

            @pl.when(u >= NU - NT)
            def _start_out():
                out_copy(t).start()

        _loop(NU, step)
        out_copy(NT - 1).wait()

    any_spec = pl.BlockSpec(memory_space=pl.ANY)
    call = pl.pallas_call(
        kernel,
        in_specs=[
            any_spec, any_spec, any_spec, any_spec, any_spec, any_spec,
        ],
        out_specs=any_spec,
        out_shape=jax.ShapeDtypeStruct((S, D), bf16),
        scratch_shapes=[
            pltpu.VMEM((S, D), bf16),
            pltpu.VMEM((D + KC, 3 * D), bf16), pltpu.VMEM((D, D), bf16),
            pltpu.VMEM((7, DHALF, 3 * DHALF), bf16), pltpu.VMEM((7, DHALF, DHALF), bf16),
            pltpu.VMEM((7, DHALF, FH), bf16), pltpu.VMEM((7, DHALF, FH), bf16), pltpu.VMEM((7, FH, DHALF), bf16),
            pltpu.VMEM((H * 40, 128), jnp.uint32),
            pltpu.VMEM((NT, TM, D), f32),
            pltpu.VMEM((2, 3 * NB, TM + HALO, 128), f32),
            pltpu.VMEM((3 * NB, TM + HALO, 128), f32),
            pltpu.VMEM((TM, D), bf16), pltpu.VMEM((2, 7, TH, DHALF), bf16),
            pltpu.VMEM((7, TH, DHALF), bf16), pltpu.VMEM((7, TH, DHALF), bf16),
            pltpu.VMEM((7, TH, FH), bf16), pltpu.VMEM((TM, D), bf16),
            pltpu.SemaphoreType.DMA((3 * NKC + 21,)),
        ],
        compiler_params=pltpu.CompilerParams(
            vmem_limit_bytes=vmem_mb * 1024 * 1024, flags=flags),
    )

    def fn(A_x, A_wqkv, A_wo, B_x, B_w1, B_w3, B_w2):
        x = A_x.reshape(S, D)
        return call(x, A_wqkv, A_wo, B_w1, B_w3, B_w2).reshape(A_x.shape)
    return jax.jit(fn)


_fn = make(flags={'XLA_TPU_EVENLY_DISTRIBUTE_CRITICAL_NODES': True})


@jax.jit
def pallas_interleave_layers__sliding_local_dilated__glu_gated_swiglu__prompt_kernel(A_x, A_wqkv, A_wo, B_x, B_w1, B_w3, B_w2):
    return _fn(A_x, A_wqkv, A_wo, B_x, B_w1, B_w3, B_w2)
```

```python
import functools
import jax
import jax.numpy as jnp
from jax.experimental import pallas as pl
from jax.experimental.pallas import tpu as pltpu

S, D, F = 2048, 1024, 3584
H, DH, W, DIL = 32, 32, 8, 2
HALO = 16
NB = D // 128
EPS = 1e-5
NEG = -1e9
SCALE = DH ** -0.5
f32, bf16 = jnp.float32, jnp.bfloat16
DHALF, FH = D // 2, F // 2


def _ln(x):
    m = jnp.mean(x, axis=-1, keepdims=True)
    c = x - m
    v = jnp.mean(c * c, axis=-1, keepdims=True)
    return c * jax.lax.rsqrt(v + EPS)


def _dot(a, b):
    return jnp.dot(a, b, preferred_element_type=f32)


def _loop(k, body, unroll=1):
    assert k % unroll == 0

    def step(i, carry):
        for j in range(unroll):
            body(i * unroll + j)
        return carry
    jax.lax.fori_loop(0, k // unroll, step, 0)


def _lhs_terms(a11, a12, a21, a22):
    return (a11 + a22, a21 + a22, a11, a22, a11 + a12, a21 - a11, a12 - a22)


def _rhs_terms(b11, b12, b21, b22):
    return (b11 + b22, b11, b12 - b22, b21 - b11, b22, b11 + b12, b21 + b22)


def _strassen(prod):
    m0, m3, m4 = prod(0), prod(3), prod(4)
    c11 = (m0 + m3) - m4 + prod(6)
    m1 = prod(1)
    c21 = m1 + m3
    m2 = prod(2)
    c12 = m2 + m4
    c22 = (m0 - m1) + m2 + prod(5)
    return c11, c12, c21, c22


SUM_SLOT = {0: 0, 2: 1, 3: 2, 5: 3, 6: 4}


def make(TM=256, FC=(512, 512, 512, 256), DC=256, WR=64, WU=8, NC=512, R=16, QC=512, LR=16, R0=64, LR0=128, KC=256, inflight=3, pitch=33, vmem_mb=120,
         flags=None, NL=2, t_slack=0, late_norm=True, t_first=False, ln_pos='U', wout=False, ufirst=True, TU=8, tree=False, PU=1, OS=1, split_ud=True, silu='tanh', border='TAL', halo_first=True, stage_in='D', NCL=512, ln_in_down=False, stop=99):
    NT = S // TM
    NU = NL * NT
    FCS = list(FC) if isinstance(FC, (list, tuple)) else [FC] * (FH // FC)
    assert sum(FCS) == FH
    FOFF = [sum(FCS[:i]) for i in range(len(FCS) + 1)]
    NFC, NNC, NQ, NP, NLR = len(FCS), DHALF // NC, 3 * DHALF // QC, TM // 2 // R, TM // 2 // LR
    NKC = D // KC
    TH = TM // 2
    NBI = TM // R0

    def kernel(x_h, wqkv_h, wo_h, w1_h, w3_h, w2_h, o_h,
               xin, wqkv, wo, wqkv7, wo7, w1, w3, w2, tbuf, xs, qkv, qkv0, x0, xa, xf, ab, hb, ob, sems):
        NPC = 3 * NKC

        def qkv_copy(i):
            blk = (pl.ds(pl.multiple_of((i // 3) * KC, KC), KC), pl.ds(pl.multiple_of((i % 3) * D, D), D))
            return pltpu.make_async_copy(wqkv_h.at[blk], wqkv.at[blk], sems.at[i])
        wo_copy = pltpu.make_async_copy(wo_h, wo, sems.at[NPC])

        def quadrant_copies(i):
            w_h, (raw, _) = ffn_w[i]
            kh, nh = raw.shape[1:]
            return [pltpu.make_async_copy(w_h.at[pl.ds(r * kh, kh), pl.ds(c * nh, nh)], raw.at[2 * r + c],
                                          sems.at[NPC + 9 + 4 * i + 2 * r + c]) for r in range(2) for c in range(2)]

        def start_dma(i):
            for cp in quadrant_copies(i):
                cp.start()

        def wait_dma(i):
            for cp in quadrant_copies(i):
                cp.wait()
        ffn_w = ((w3_h, w3), (w1_h, w1), (w2_h, w2))

        def rhs_terms(w):
            raw, sums = w
            per = raw.shape[1] // WR

            def body(r):
                p, rs = r // per, row_slice(r % per, WR)
                quads = (raw[i, rs, pl.ds(pl.multiple_of(p * 128, 128), 128)].astype(f32) for i in range(4))
                for i, term in enumerate(_rhs_terms(*quads)):
                    if i in SUM_SLOT:
                        sums[SUM_SLOT[i], p, rs, :] = term.astype(bf16)
            _loop(sums.shape[1] * per, body, WU)

        def ffn_rhs(w, i, c0, cols):
            raw, sums = w
            if i in SUM_SLOT:
                return panels(sums, SUM_SLOT[i], c0 // 128, cols // 128)
            return raw[0 if i == 1 else 3, :, pl.ds(c0, cols)]

        def proj_terms(dst, src):
            per = DHALF // WR

            def body(r):
                p, r = r // per, r % per
                col = (p // (NB // 2)) * D + (p % (NB // 2)) * 128
                quads = (src[row_slice(i * per + r, WR), pl.ds(pl.multiple_of(col + j * DHALF, 128), 128)].astype(f32)
                         for i in range(2) for j in range(2))
                for i, term in enumerate(_rhs_terms(*quads)):
                    dst[i, p, row_slice(r, WR), :] = term.astype(bf16)
            _loop(dst.shape[1] * per, body, WU)

        def panels(w, i, p0, count):
            return jnp.concatenate([w[i, p0 + p] for p in range(count)], axis=1)

        def x_copy(i, r0, rows):
            return pltpu.make_async_copy(x_h.at[pl.ds(r0, rows)], xin.at[pl.ds(r0, rows)], sems.at[NPC + 4 + i])
        x_copies = [x_copy(0, 0, TM), x_copy(1, TM, 3 * TM), x_copy(2, 4 * TM, S - 4 * TM)]

        def permute_qkv(src_r, dst_r, m):
            al = lambda v, k: v if isinstance(v, int) else pl.multiple_of(v, k)
            cs = pl.ds(al(m * D, D), D)
            u = pltpu.bitcast(wqkv[pl.ds(al(src_r, KC), KC), cs], jnp.uint32).T
            for h in range(H):
                tbuf[pl.ds(h * pitch, DH), :] = u[h * DH:(h + 1) * DH]
            p = jnp.concatenate([tbuf[pl.ds(d, H, stride=pitch), :] for d in range(DH)], axis=0)
            wqkv[pl.ds(al(dst_r, KC), KC), cs] = pltpu.bitcast(p.T, bf16)

        def permute_wo(j):
            cs = pl.ds(pl.multiple_of(j * 128, 128), 128)
            for h in range(H):
                tbuf[pl.ds(h * pitch, DH), :] = pltpu.bitcast(wo[pl.ds(h * DH, DH), cs].astype(f32), jnp.uint32)
            for d in range(DH):
                wo[pl.ds(d * H, H), cs] = pltpu.bitcast(tbuf[pl.ds(d, H, stride=pitch), :], f32).astype(bf16)

        def row_slice(r, rows):
            return pl.ds(r * rows if isinstance(r, int) else pl.multiple_of(r * rows, rows), rows)

        def store_lhs(dst, rs, top, bot):
            terms = _lhs_terms(top[:, :DHALF], top[:, DHALF:], bot[:, :DHALF], bot[:, DHALF:])
            for i, term in enumerate(terms):
                dst[i, rs, :] = term.astype(bf16)

        def ln_ffn(tile, r, rows=LR):
            top, bot = (_ln(xs[tile, row_slice(k, rows), :]) for k in (r, TH // rows + r))
            store_lhs(xf, row_slice(r, rows), top, bot)

        def resid(u, r, rows, cs=slice(None)):
            x0 = xin[row_slice((u % NT) * (TM // rows) + r, rows), cs].astype(f32)
            if isinstance(u, int):
                assert u < NT
                return x0
            return jnp.where(u < NT, x0, xs[u % NT, row_slice(r, rows), cs])

        def ln_attn(u, r, rows=LR):
            top, bot = (_ln(resid(u, k, rows)) for k in (r, TH // rows + r))
            store_lhs(xa.at[u % 2], row_slice(r, rows), top, bot)

        def ln_first(r, rows):
            x0[row_slice(r, rows), :] = _ln(resid(0, r, rows)).astype(bf16)

        def a_dot(slot, c, cols):
            out = _strassen(lambda i: _dot(xa[slot, i], panels(wqkv7, i, c * (cols // 128), cols // 128)))
            for jj in range(cols // 128):
                k = c * (cols // 128) + jj
                slab = (k // (NB // 2)) * NB + k % (NB // 2)
                for i, o in enumerate(out):
                    qkv[slot, slab + (i % 2) * (NB // 2), pl.ds(HALO + (i // 2) * TH, TH), :] = o[:, jj * 128:(jj + 1) * 128]

        def a_dot_partial(c, m):
            ks = pl.ds(pl.multiple_of(c * KC, KC), KC)
            res = _dot(x0[:, ks], wqkv[ks, pl.ds(pl.multiple_of(m * D, D), D)])
            for j in range(NB):
                dst = (m * NB + j, pl.ds(HALO, TM), slice(None))
                part = res[:, j * 128:(j + 1) * 128]
                qkv0[dst] = jnp.where(c == 0, part, qkv0[dst] + part)

        def halo_carry(dst, src):
            for j in range(NB, 3 * NB):
                dst[j, pl.ds(0, HALO), :] = src[j, pl.ds(TM, HALO), :]

        def halo_init(buf, t):
            for j in range(NB, 3 * NB):
                first = jnp.broadcast_to(buf[j, pl.ds(HALO, 1), :], (HALO, 128))
                buf[j, pl.ds(0, HALO), :] = jnp.where(t == 0, first, buf[j, pl.ds(0, HALO), :])

        def attend(buf, t, p, R):
            static = isinstance(p, int)
            r0 = p * R if static else pl.multiple_of(p * R, R)
            lg = [None] * W
            q = [buf[j, pl.ds(r0 + HALO, R), :] for j in range(NB)]
            for j, w in ([(j, w) for w in range(W) for j in range(NB)] if wout else [(j, w) for j in range(NB) for w in range(W)]):
                pr = q[j] * buf[NB + j, pl.ds(r0 + HALO - DIL * w, R), :]
                lg[w] = pr if j == 0 else lg[w] + pr
            for w in range(W):
                a = lg[w]
                a = a + pltpu.roll(a, 64, 1)
                a = (a + pltpu.roll(a, 32, 1)) * SCALE
                if (not static) or r0 < DIL * w:
                    pos = t * TM + r0 + jax.lax.broadcasted_iota(jnp.int32, (R, 128), 0)
                    a = jnp.where(pos >= DIL * w, a, NEG)
                lg[w] = a
            mx = functools.reduce(jnp.maximum, lg)
            e = [jnp.exp(a - mx) for a in lg]
            inv = 1.0 / functools.reduce(lambda a, b: a + b, e)
            pw = e if late_norm else [a * inv for a in e]
            out = []
            for j in range(NB):
                acc = None
                for w in range(W):
                    pr = pw[w] * buf[2 * NB + j, pl.ds(r0 + HALO - DIL * w, R), :]
                    acc = pr if acc is None else acc + pr
                out.append(acc * inv if late_norm else acc)
            return jnp.concatenate(out, axis=1)

        def t_piece(buf, t, p, R=R):
            store_lhs(ab, row_slice(p, R), attend(buf, t, p, R), attend(buf, t, TH // R + p, R))

        def o_dot(u, c, cols):
            c0 = c * cols if isinstance(c, int) else pl.multiple_of(c * cols, cols)
            out = _strassen(lambda i: _dot(ab[i], panels(wo7, i, c * (cols // 128), cols // 128)))
            for i, o in enumerate(out):
                cs = pl.ds((i % 2) * DHALF + c0, cols)
                xs[u % NT, row_slice(i // 2, TH), cs] = resid(u, i // 2, TH, cs) + o

        def f_up(c):
            cs = pl.ds(FOFF[c], FCS[c])
            if ufirst: up = _strassen(lambda i: _dot(xf[i], ffn_rhs(w3, i, FOFF[c], FCS[c])))
            gate = _strassen(lambda i: _dot(xf[i], ffn_rhs(w1, i, FOFF[c], FCS[c])))
            if not ufirst: up = _strassen(lambda i: _dot(xf[i], ffn_rhs(w3, i, FOFF[c], FCS[c])))
            h = []
            for g, u in zip(gate, up):
                hg = 0.5 * g
                h.append((hg * jnp.tanh(hg) + hg) * u)
            for i, term in enumerate(_lhs_terms(*h)):
                hb[i, :, cs] = term.astype(bf16)

        def f_down(tp, c):
            out = _strassen(lambda i: _dot(hb[i], ffn_rhs(w2, i, c * DC, DC)))
            for i, o in enumerate(out):
                rs, cs = pl.ds((i // 2) * TH, TH), pl.ds((i % 2) * DHALF + c * DC, DC)
                y = xs[tp, rs, cs] + o
                xs[tp, rs, cs] = y
                ob[rs, cs] = y.astype(ob.dtype)

        def spread(total, c, slots):
            return range(min(total, (total * c) // slots), min(total, (total * (c + 1)) // slots))

        with jax.named_scope('_prologue'):
            x_copies[0].start()
            qkv_copy(0).start()
            x_copies[0].wait()
            for i in range(1, inflight):
                qkv_copy(i).start()
            _loop(TM // LR0, lambda r: ln_first(r, LR0))

            def dma(i):
                @pl.when(i < NPC)
                def _():
                    qkv_copy(i).wait()

                @pl.when(i + inflight < NPC)
                def _():
                    qkv_copy(i + inflight).start()

                @pl.when(i + inflight == NPC)
                def _():
                    x_copies[1].start()

                @pl.when(i == NPC - 1)
                def _():
                    wo_copy.start()

            def piece(k):
                for i in range(PU):
                    dma(k * PU + i + (PU > 1))
                for i in range(PU):
                    i = k * PU + i + (PU > 1)
                    ip = jnp.maximum(i - 1, 0)
                    a_dot_partial(ip // 3, ip % 3)
                    permute_qkv(jnp.minimum(i // 3, NKC - 1) * KC, (i // 3) * KC, i % 3)
            if PU > 1:
                dma(jnp.int32(0))
                permute_qkv(0, 0, 0)
                _loop(NPC // PU, piece)
            else:
                _loop(NPC + 1, piece)

        with jax.named_scope('_prologue2'):
            halo_init(qkv0, 0)
            halo_carry(qkv.at[1], qkv0)
            x_copies[1].wait()
            start_dma(0)
            start_dma(1)
            _loop(TM // LR0, lambda r: ln_attn(1, r, LR0 // 2))
            proj_terms(wqkv7, wqkv)

            def piece(p):
                for ch in border:
                    if ch == 'T': t_piece(qkv0, 0, p, R0 // 2)
                    if ch == 'P': permute_wo(p)
                    if ch == 'L': ln_attn(2, p, R0 // 2)
                    if ch == 'A': a_dot(1, p, 3 * DHALF // NBI)
            _loop(NBI, piece)
            wo_copy.wait()
            _loop(NB, permute_wo)
            proj_terms(wo7, wo)

        def out_copy(tile):
            return pltpu.make_async_copy(ob, o_h.at[row_slice(tile, TM)], sems.at[NPC + 8])

        def step(u):
            t, t1 = u % NT, (u + 1) % NT
            s0, s1 = u % 2, (u + 1) % 2

            @pl.when(u + 2 < NU)
            def _oproj_qkv():
                halo_carry(qkv.at[s0], qkv.at[s1])
                for c in range(NNC):
                    o_dot(u, c, NC)
                for c in range(NQ):
                    a_dot(s0, c, QC)
                    for r in spread(NLR, c, NQ):
                        ln_ffn(t, r)

            @pl.when(u + 2 >= NU)
            def _oproj():
                for c in range(DHALF // NCL):
                    o_dot(u, c, NCL)
                _loop(TM // LR0, lambda r: ln_ffn(t, r, LR0 // 2))

            @pl.when(u == 0)
            def _wait_up():
                wait_dma(0)
                rhs_terms(w3)
                wait_dma(1)
                x_copies[2].start()
                start_dma(2)
                rhs_terms(w1)

            @pl.when(u == 1)
            def _wait_x():
                x_copies[2].wait()

            @pl.when(u > NU - NT)
            def _wait_out():
                out_copy(t).wait()

            halo_init(qkv.at[s1], t1)
            for c in range(NFC):
                if not t_first: f_up(c)
                for p in range(min(TU, TU * FOFF[c] // (FH - t_slack)), min(TU, TU * FOFF[c + 1] // (FH - t_slack))):
                    t_piece(qkv.at[s1], t1, p)
                if ln_pos == 'U':
                    for r in range(min(NLR, NLR * FOFF[c] // (FH - t_slack)), min(NLR, NLR * FOFF[c + 1] // (FH - t_slack))):
                        ln_attn(u + 3, r)
                if t_first: f_up(c)

            if split_ud:
                @pl.when(u == 0)
                def _wait_down():
                    wait_dma(2)
                    rhs_terms(w2)

            for c in range(DHALF // DC):
                f_down(t, c)
                for p in spread(NP - TU, c, DHALF // DC):
                    t_piece(qkv.at[s1], t1, TU + p)
                if ln_pos == 'D':
                    for r in spread(NLR, c, DHALF // DC):
                        ln_attn(u + 3, r)

            @pl.when(u >= NU - NT)
            def _start_out():
                out_copy(t).start()

        _loop(NU, step)
        out_copy(NT - 1).wait()

    def ffn_scratch(kh, nh):
        return (pltpu.VMEM((4, kh, nh), bf16), pltpu.VMEM((5, nh // 128, kh, 128), bf16))

    any_spec = pl.BlockSpec(memory_space=pl.ANY)
    call = pl.pallas_call(
        kernel,
        in_specs=[
            any_spec, any_spec, any_spec, any_spec, any_spec, any_spec,
        ],
        out_specs=any_spec,
        out_shape=jax.ShapeDtypeStruct((S, D), bf16),
        scratch_shapes=[
            pltpu.VMEM((S, D), bf16),
            pltpu.VMEM((D + KC, 3 * D), bf16), pltpu.VMEM((D, D), bf16),
            pltpu.VMEM((7, 3 * DHALF // 128, DHALF, 128), bf16), pltpu.VMEM((7, DHALF // 128, DHALF, 128), bf16),
            ffn_scratch(DHALF, FH), ffn_scratch(DHALF, FH), ffn_scratch(FH, DHALF),
            pltpu.VMEM((H * 40, 128), jnp.uint32),
            pltpu.VMEM((NT, TM, D), f32),
            pltpu.VMEM((2, 3 * NB, TM + HALO, 128), f32),
            pltpu.VMEM((3 * NB, TM + HALO, 128), f32),
            pltpu.VMEM((TM, D), bf16), pltpu.VMEM((2, 7, TH, DHALF), bf16),
            pltpu.VMEM((7, TH, DHALF), bf16), pltpu.VMEM((7, TH, DHALF), bf16),
            pltpu.VMEM((7, TH, FH), bf16), pltpu.VMEM((TM, D), bf16),
            pltpu.SemaphoreType.DMA((3 * NKC + 21,)),
        ],
        compiler_params=pltpu.CompilerParams(
            vmem_limit_bytes=vmem_mb * 1024 * 1024, flags=flags),
    )

    def fn(A_x, A_wqkv, A_wo, B_x, B_w1, B_w3, B_w2):
        x = A_x.reshape(S, D)
        return call(x, A_wqkv, A_wo, B_w1, B_w3, B_w2).reshape(A_x.shape)
    return jax.jit(fn)


_fn = make(flags={'XLA_TPU_EVENLY_DISTRIBUTE_CRITICAL_NODES': True})


@jax.jit
def pallas_interleave_layers__sliding_local_dilated__glu_gated_swiglu__prompt_kernel(A_x, A_wqkv, A_wo, B_x, B_w1, B_w3, B_w2):
    return _fn(A_x, A_wqkv, A_wo, B_x, B_w1, B_w3, B_w2)
```

```python
import functools

import jax
import jax.numpy as jnp
from jax.experimental import pallas as pl
from jax.experimental.pallas import tpu as pltpu

S, D, F = 2048, 1024, 3584
H, DH, W, DIL = 32, 32, 8, 2
EPS = 1e-5
NEG = -1e9
SCALE = DH ** -0.5
f32, bf16 = jnp.float32, jnp.bfloat16

TM = 256
TH, DHALF, FH = TM // 2, D // 2, F // 2
NT = S // TM
NU = 2 * NT
NB = D // 128
HALO = 16
KC = 256
NPC = 3 * (D // KC)
INFLIGHT = 3
PITCH = DH + 1
R = 16
NR = TH // R
R0, LR0 = 32, 128
WR, WU = 64, 8
UP_COLS = (512, 512, 512, 256)
PROJ_COLS, DOWN_COLS = 512, 256
SUM_SLOT = {0: 0, 2: 1, 3: 2, 5: 3, 6: 4}


def _ln(x):
    c = x - jnp.mean(x, axis=-1, keepdims=True)
    return c * jax.lax.rsqrt(jnp.mean(c * c, axis=-1, keepdims=True) + EPS)


def _dot(a, b):
    return jnp.dot(a, b, preferred_element_type=f32)


def _loop(count, body, unroll=1):
    def step(i, carry):
        for j in range(unroll):
            body(i * unroll + j)
        return carry
    jax.lax.fori_loop(0, count // unroll, step, 0)


def _block(i, size, align=None):
    return pl.ds(i * size if isinstance(i, int) else pl.multiple_of(i * size, align or size), size)


def _share(total, lo, hi, whole):
    return range(total * lo // whole, total * hi // whole)


def _lhs_terms(a11, a12, a21, a22):
    return (a11 + a22, a21 + a22, a11, a22, a11 + a12, a21 - a11, a12 - a22)


def _rhs_terms(b11, b12, b21, b22):
    return (b11 + b22, b11, b12 - b22, b21 - b11, b22, b11 + b12, b21 + b22)


def _strassen(prod):
    m0, m3, m4 = prod(0), prod(3), prod(4)
    c11 = (m0 + m3) - m4 + prod(6)
    m1 = prod(1)
    c21 = m1 + m3
    m2 = prod(2)
    c12 = m2 + m4
    c22 = (m0 - m1) + m2 + prod(5)
    return c11, c12, c21, c22


def _kernel(x_h, wqkv_h, wo_h, w1_h, w3_h, w2_h, o_h,
            xin, wqkv, wo, wqkv7, wo7, w1, w3, w2, tbuf, tbuf2, xs, qkv, qkv0, x0, xa, xf, ab, hb, ob, sems):
    def qkv_copy(i):
        blk = (_block(i // 3, KC), _block(i % 3, D))
        return pltpu.make_async_copy(wqkv_h.at[blk], wqkv.at[blk], sems.at[i])

    wo_copy = pltpu.make_async_copy(wo_h, wo, sems.at[NPC])
    x_copies = [
        pltpu.make_async_copy(x_h.at[pl.ds(r0, rows)], xin.at[pl.ds(r0, rows)], sems.at[NPC + 1 + i])
        for i, (r0, rows) in enumerate(((0, TM), (TM, 3 * TM), (4 * TM, S - 4 * TM)))]

    def out_copy(tile):
        return pltpu.make_async_copy(ob, o_h.at[_block(tile, TM)], sems.at[NPC + 4])

    def quadrant_copies(w_h, w, sem0):
        raw = w[0]
        kh, nh = raw.shape[1:]
        return [pltpu.make_async_copy(w_h.at[pl.ds(r * kh, kh), pl.ds(c * nh, nh)], raw.at[2 * r + c],
                                      sems.at[sem0 + 2 * r + c]) for r in range(2) for c in range(2)]

    w3_copies = quadrant_copies(w3_h, w3, NPC + 5)
    w1_copies = quadrant_copies(w1_h, w1, NPC + 9)
    w2_copies = quadrant_copies(w2_h, w2, NPC + 13)

    def permute_qkv(src, dst, m):
        cs = _block(m, D)
        u = pltpu.bitcast(wqkv[_block(src, KC), cs], jnp.uint32).T
        for h in range(H):
            tbuf[pl.ds(h * PITCH, DH), :] = u[h * DH:(h + 1) * DH]
        p = jnp.concatenate([tbuf[pl.ds(d, H, stride=PITCH), :] for d in range(DH)], axis=0)
        wqkv[_block(dst, KC), cs] = pltpu.bitcast(p.T, bf16)

    def qkv_terms():
        per = DHALF // WR

        def body(i):
            p, r = i // per, i % per
            col = (p // (NB // 2)) * NB + p % (NB // 2)
            quads = (wqkv[_block(a * per + r, WR), _block(col + b * (NB // 2), 128)].astype(f32)
                     for a in range(2) for b in range(2))
            for k, term in enumerate(_rhs_terms(*quads)):
                wqkv7[k, p, _block(r, WR), :] = term.astype(bf16)
        _loop(wqkv7.shape[1] * per, body, WU)

    def wo_terms(j):
        for half, buf in enumerate((tbuf, tbuf2)):
            cs = _block(half * (NB // 2) + j, 128)
            for h in range(H):
                buf[pl.ds(h * PITCH, DH), :] = pltpu.bitcast(wo[pl.ds(h * DH, DH), cs].astype(f32), jnp.uint32)
        for d in range(DH // 2):
            quads = (pltpu.bitcast(buf[pl.ds(dd, H, stride=PITCH), :], f32)
                     for dd in (d, d + DH // 2) for buf in (tbuf, tbuf2))
            for k, term in enumerate(_rhs_terms(*quads)):
                wo7[k, j, pl.ds(d * H, H), :] = term.astype(bf16)

    def ffn_terms(w):
        raw, sums = w
        per = raw.shape[1] // WR

        def body(i):
            p, rs = i // per, _block(i % per, WR)
            quads = (raw[q, rs, _block(p, 128)].astype(f32) for q in range(4))
            for k, term in enumerate(_rhs_terms(*quads)):
                if k in SUM_SLOT:
                    sums[SUM_SLOT[k], p, rs, :] = term.astype(bf16)
        _loop(sums.shape[1] * per, body, WU)

    def panels(w, k, first, count):
        return jnp.concatenate([w[k, first + p] for p in range(count)], axis=1)

    def ffn_rhs(w, k, c0, cols):
        raw, sums = w
        if k in SUM_SLOT:
            return panels(sums, SUM_SLOT[k], c0 // 128, cols // 128)
        return raw[0 if k == 1 else 3, :, pl.ds(c0, cols)]

    def store_lhs(dst, rs, top, bot):
        terms = _lhs_terms(top[:, :DHALF], top[:, DHALF:], bot[:, :DHALF], bot[:, DHALF:])
        for k, term in enumerate(terms):
            dst[k, rs, :] = term.astype(bf16)

    def resid(u, r, rows, cs=slice(None)):
        first = xin[_block((u % NT) * (TM // rows) + r, rows), cs].astype(f32)
        if isinstance(u, int):
            return first
        return jnp.where(u < NT, first, xs[u % NT, _block(r, rows), cs])

    def ln_attn(u, r, rows):
        top, bot = (_ln(resid(u, k, rows)) for k in (r, TH // rows + r))
        store_lhs(xa.at[u % 2], _block(r, rows), top, bot)

    def ln_ffn(tile, r, rows):
        top, bot = (_ln(xs[tile, _block(k, rows), :]) for k in (r, TH // rows + r))
        store_lhs(xf, _block(r, rows), top, bot)

    def halo_carry(dst, src):
        for j in range(NB, 3 * NB):
            dst[j, pl.ds(0, HALO), :] = src[j, pl.ds(TM, HALO), :]

    def halo_init(buf, tile):
        for j in range(NB, 3 * NB):
            first = jnp.broadcast_to(buf[j, pl.ds(HALO, 1), :], (HALO, 128))
            buf[j, pl.ds(0, HALO), :] = jnp.where(tile == 0, first, buf[j, pl.ds(0, HALO), :])

    def attend(buf, tile, r, rows):
        static = isinstance(r, int)
        r0 = r * rows if static else pl.multiple_of(r * rows, rows)
        logits = [None] * W
        for j in range(NB):
            q = buf[j, pl.ds(r0 + HALO, rows), :]
            for w in range(W):
                qk = q * buf[NB + j, pl.ds(r0 + HALO - DIL * w, rows), :]
                logits[w] = qk if j == 0 else logits[w] + qk
        for w in range(W):
            a = logits[w]
            a = a + pltpu.roll(a, 2 * H, 1)
            a = (a + pltpu.roll(a, H, 1)) * SCALE
            if not static or r0 < DIL * w:
                pos = tile * TM + r0 + jax.lax.broadcasted_iota(jnp.int32, (rows, 128), 0)
                a = jnp.where(pos >= DIL * w, a, NEG)
            logits[w] = a
        mx = functools.reduce(jnp.maximum, logits)
        e = [jnp.exp(a - mx) for a in logits]
        inv = 1.0 / functools.reduce(jnp.add, e)
        out = []
        for j in range(NB):
            acc = None
            for w in range(W):
                pv = e[w] * buf[2 * NB + j, pl.ds(r0 + HALO - DIL * w, rows), :]
                acc = pv if acc is None else acc + pv
            out.append(acc * inv)
        return jnp.concatenate(out, axis=1)

    def attention(buf, tile, r, rows):
        store_lhs(ab, _block(r, rows), attend(buf, tile, r, rows), attend(buf, tile, TH // rows + r, rows))

    def qkv_first(c, m):
        res = _dot(x0[:, _block(c, KC)], wqkv[_block(c, KC), _block(m, D)])
        for j in range(NB):
            dst = (m * NB + j, pl.ds(HALO, TM), slice(None))
            part = res[:, j * 128:(j + 1) * 128]
            qkv0[dst] = jnp.where(c == 0, part, qkv0[dst] + part)

    def qkv_proj(slot, c, cols):
        count = cols // 128
        out = _strassen(lambda k: _dot(xa[slot, k], panels(wqkv7, k, c * count, count)))
        for j in range(count):
            p = c * count + j
            slab = (p // (NB // 2)) * NB + p % (NB // 2)
            for i, o in enumerate(out):
                qkv[slot, slab + (i % 2) * (NB // 2), pl.ds(HALO + (i // 2) * TH, TH), :] = o[:, j * 128:(j + 1) * 128]

    def out_proj(u):
        out = _strassen(lambda k: _dot(ab[k], panels(wo7, k, 0, NB // 2)))
        for i, o in enumerate(out):
            cs = _block(i % 2, DHALF)
            xs[u % NT, _block(i // 2, TH), cs] = resid(u, i // 2, TH, cs) + o

    def ffn_up(c0, cols):
        up = _strassen(lambda k: _dot(xf[k], ffn_rhs(w3, k, c0, cols)))
        gate = _strassen(lambda k: _dot(xf[k], ffn_rhs(w1, k, c0, cols)))
        hidden = []
        for g, u in zip(gate, up):
            half = 0.5 * g
            hidden.append((half * jnp.tanh(half) + half) * u)
        for k, term in enumerate(_lhs_terms(*hidden)):
            hb[k, :, pl.ds(c0, cols)] = term.astype(bf16)

    def ffn_down(tile, c0, cols):
        out = _strassen(lambda k: _dot(hb[k], ffn_rhs(w2, k, c0, cols)))
        for i, o in enumerate(out):
            rs, cs = _block(i // 2, TH), pl.ds((i % 2) * DHALF + c0, cols)
            y = xs[tile, rs, cs] + o
            xs[tile, rs, cs] = y
            ob[rs, cs] = y.astype(ob.dtype)

    x_copies[0].start()
    qkv_copy(0).start()
    x_copies[0].wait()
    for i in range(1, INFLIGHT):
        qkv_copy(i).start()

    def ln_first(r):
        x0[_block(r, LR0), :] = _ln(resid(0, r, LR0)).astype(bf16)
    _loop(TM // LR0, ln_first)

    def first_piece(i):
        @pl.when(i < NPC)
        def _():
            qkv_copy(i).wait()

        @pl.when(i + INFLIGHT < NPC)
        def _():
            qkv_copy(i + INFLIGHT).start()

        @pl.when(i + INFLIGHT == NPC)
        def _():
            x_copies[1].start()

        @pl.when(i == NPC - 1)
        def _():
            wo_copy.start()
        prev = jnp.maximum(i - 1, 0)
        qkv_first(prev // 3, prev % 3)
        permute_qkv(jnp.minimum(i // 3, D // KC - 1), i // 3, i % 3)
    _loop(NPC + 1, first_piece)

    halo_init(qkv0, 0)
    halo_carry(qkv.at[1], qkv0)
    x_copies[1].wait()
    for cp in w3_copies + w1_copies:
        cp.start()
    _loop(TM // LR0, lambda r: ln_attn(1, r, LR0 // 2))
    qkv_terms()

    def second_piece(r):
        attention(qkv0, 0, r, R0)
        qkv_proj(1, r, 3 * DHALF // (TH // R0))
        ln_attn(2, r, R0)
    _loop(TH // R0, second_piece)
    wo_copy.wait()
    _loop(NB // 2, wo_terms)

    def step(u):
        tile, ahead = u % NT, (u + 1) % NT
        s0, s1 = u % 2, (u + 1) % 2

        @pl.when(u + 2 < NU)
        def _():
            halo_carry(qkv.at[s0], qkv.at[s1])
            out_proj(u)
            chunks = 3 * DHALF // PROJ_COLS
            for c in range(chunks):
                qkv_proj(s0, c, PROJ_COLS)
                for r in _share(NR, c, c + 1, chunks):
                    ln_ffn(tile, r, R)

        @pl.when(u + 2 >= NU)
        def _():
            out_proj(u)
            _loop(TM // LR0, lambda r: ln_ffn(tile, r, LR0 // 2))

        @pl.when(u == 0)
        def _():
            for cp in w3_copies:
                cp.wait()
            ffn_terms(w3)
            for cp in w1_copies:
                cp.wait()
            x_copies[2].start()
            for cp in w2_copies:
                cp.start()
            ffn_terms(w1)

        @pl.when(u == 1)
        def _():
            x_copies[2].wait()

        @pl.when(u > NU - NT)
        def _():
            out_copy(tile).wait()

        halo_init(qkv.at[s1], ahead)
        c0 = 0
        for cols in UP_COLS:
            ffn_up(c0, cols)
            for r in _share(NR, c0, c0 + cols, FH):
                attention(qkv.at[s1], ahead, r, R)
            for r in _share(NR, c0, c0 + cols, FH):
                ln_attn(u + 3, r, R)
            c0 += cols

        @pl.when(u == 0)
        def _():
            for cp in w2_copies:
                cp.wait()
            ffn_terms(w2)

        for c0 in range(0, DHALF, DOWN_COLS):
            ffn_down(tile, c0, DOWN_COLS)

        @pl.when(u >= NU - NT)
        def _():
            out_copy(tile).start()

    _loop(NU, step)
    out_copy(NT - 1).wait()


def _ffn_scratch(kh, nh):
    return (pltpu.VMEM((4, kh, nh), bf16),
            pltpu.VMEM((5, nh // 128, kh, 128), bf16))


@jax.jit
def pallas_interleave_layers__sliding_local_dilated__glu_gated_swiglu__prompt_kernel(
    A_x: jax.Array,
    A_wqkv: jax.Array,
    A_wo: jax.Array,
    B_x: jax.Array,
    B_w1: jax.Array,
    B_w3: jax.Array,
    B_w2: jax.Array,
):
    del B_x
    hbm = pl.BlockSpec(memory_space=pl.ANY)
    out = pl.pallas_call(
        _kernel,
        in_specs=[hbm] * 6,
        out_specs=hbm,
        out_shape=jax.ShapeDtypeStruct((S, D), bf16),
        scratch_shapes=[
            pltpu.VMEM((S, D), bf16),
            pltpu.VMEM((D + KC, 3 * D), bf16),
            pltpu.VMEM((D, D), bf16),
            pltpu.VMEM((7, 3 * NB // 2, DHALF, 128), bf16),
            pltpu.VMEM((7, NB // 2, DHALF, 128), bf16),
            _ffn_scratch(DHALF, FH), _ffn_scratch(DHALF, FH), _ffn_scratch(FH, DHALF),
            pltpu.VMEM((H * 40, 128), jnp.uint32),
            pltpu.VMEM((H * 40, 128), jnp.uint32),
            pltpu.VMEM((NT, TM, D), f32),
            pltpu.VMEM((2, 3 * NB, TM + HALO, 128), f32),
            pltpu.VMEM((3 * NB, TM + HALO, 128), f32),
            pltpu.VMEM((TM, D), bf16),
            pltpu.VMEM((2, 7, TH, DHALF), bf16),
            pltpu.VMEM((7, TH, DHALF), bf16),
            pltpu.VMEM((7, TH, DHALF), bf16),
            pltpu.VMEM((7, TH, FH), bf16),
            pltpu.VMEM((TM, D), bf16),
            pltpu.SemaphoreType.DMA((NPC + 17,)),
        ],
        compiler_params=pltpu.CompilerParams(
            vmem_limit_bytes=120 * 1024 * 1024,
            flags={"XLA_TPU_EVENLY_DISTRIBUTE_CRITICAL_NODES": True},
        ),
    )(A_x.reshape(S, D), A_wqkv, A_wo, B_w1, B_w3, B_w2)
    return out.reshape(A_x.shape)
```

```python
import functools

import jax
import jax.numpy as jnp
from jax.experimental import pallas as pl
from jax.experimental.pallas import tpu as pltpu

S, D, F = 2048, 1024, 3584
H, DH, W, DIL = 32, 32, 8, 2
EPS = 1e-5
NEG = -1e9
SCALE = DH ** -0.5
f32, bf16 = jnp.float32, jnp.bfloat16

TM = 256
TH, DHALF, FH = TM // 2, D // 2, F // 2
NT = S // TM
NU = 2 * NT
NB = D // 128
HALO = 16
KC = 256
NPC = 3 * (D // KC)
INFLIGHT = 3
PITCH = DH + 1
R = 16
NR = TH // R
R0 = 32
LR0 = 256
WR = 64
WU = 16
UP_COLS = (512, 512, 512, 256)
PROJ_COLS = 512
DOWN_COLS = 256
SUM_SLOT = {0: 0, 2: 1, 3: 2, 5: 3, 6: 4}


def _ln(x):
    c = x - jnp.mean(x, axis=-1, keepdims=True)
    return c * jax.lax.rsqrt(jnp.mean(c * c, axis=-1, keepdims=True) + EPS)


def _dot(a, b):
    return jnp.dot(a, b, preferred_element_type=f32)


def _loop(count, body, unroll=1):
    def step(i, carry):
        for j in range(unroll):
            body(i * unroll + j)
        return carry
    jax.lax.fori_loop(0, count // unroll, step, 0)


def _block(i, size, align=None):
    return pl.ds(i * size if isinstance(i, int) else pl.multiple_of(i * size, align or size), size)


def _share(total, lo, hi, whole):
    return range(total * lo // whole, total * hi // whole)


def _lhs_terms(a11, a12, a21, a22):
    return (a11 + a22, a21 + a22, a11, a22, a11 + a12, a21 - a11, a12 - a22)


def _rhs_terms(b11, b12, b21, b22):
    return (b11 + b22, b11, b12 - b22, b21 - b11, b22, b11 + b12, b21 + b22)


def _strassen(prod):
    m0, m3, m4 = prod(0), prod(3), prod(4)
    c11 = (m0 + m3) - m4 + prod(6)
    m1 = prod(1)
    c21 = m1 + m3
    m2 = prod(2)
    c12 = m2 + m4
    c22 = (m0 - m1) + m2 + prod(5)
    return c11, c12, c21, c22


def _kernel(x_h, wqkv_h, wo_h, w1_h, w3_h, w2_h, o_h,
            xin, wqkv, wo, wqkv7, wo7, w1, w3, w2, tbuf, tbuf2, xs, qkv, qkv0, x0, xa, xf, ab, hb, ob, sems):
    def qkv_copy(i):
        blk = (_block(i // 3, KC), _block(i % 3, D))
        return pltpu.make_async_copy(wqkv_h.at[blk], wqkv.at[blk], sems.at[i])

    wo_copy = pltpu.make_async_copy(wo_h, wo, sems.at[NPC])
    x_copies = [
        pltpu.make_async_copy(x_h.at[pl.ds(r0, rows)], xin.at[pl.ds(r0, rows)], sems.at[NPC + 1 + i])
        for i, (r0, rows) in enumerate(((0, TM), (TM, 3 * TM), (4 * TM, S - 4 * TM)))]

    def out_copy(tile):
        return pltpu.make_async_copy(ob, o_h.at[_block(tile, TM)], sems.at[NPC + 4])

    def quadrant_copies(w_h, w, sem0):
        raw = w[0]
        kh, nh = raw.shape[1:]
        return [pltpu.make_async_copy(w_h.at[pl.ds(r * kh, kh), pl.ds(c * nh, nh)], raw.at[2 * r + c],
                                      sems.at[sem0 + 2 * r + c]) for r in range(2) for c in range(2)]

    w3_copies = quadrant_copies(w3_h, w3, NPC + 5)
    w1_copies = quadrant_copies(w1_h, w1, NPC + 9)
    w2_copies = quadrant_copies(w2_h, w2, NPC + 13)

    def permute_qkv(src, dst, m):
        cs = _block(m, D)
        u = pltpu.bitcast(wqkv[_block(src, KC), cs], jnp.uint32).T
        for h in range(H):
            tbuf[pl.ds(h * PITCH, DH), :] = u[h * DH:(h + 1) * DH]
        p = jnp.concatenate([tbuf[pl.ds(d, H, stride=PITCH), :] for d in range(DH)], axis=0)
        wqkv[_block(dst, KC), cs] = pltpu.bitcast(p.T, bf16)

    def qkv_terms():
        per = DHALF // WR

        def body(i):
            p, r = i // per, i % per
            col = (p // (NB // 2)) * NB + p % (NB // 2)
            quads = (wqkv[_block(a * per + r, WR), _block(col + b * (NB // 2), 128)].astype(f32)
                     for a in range(2) for b in range(2))
            for k, term in enumerate(_rhs_terms(*quads)):
                wqkv7[k, p, _block(r, WR), :] = term.astype(bf16)
        _loop(wqkv7.shape[1] * per, body, WU)

    def wo_terms(j):
        for half, buf in enumerate((tbuf, tbuf2)):
            cs = _block(half * (NB // 2) + j, 128)
            for h in range(H):
                buf[pl.ds(h * PITCH, DH), :] = pltpu.bitcast(wo[pl.ds(h * DH, DH), cs].astype(f32), jnp.uint32)
        for d in range(DH // 2):
            quads = (pltpu.bitcast(buf[pl.ds(dd, H, stride=PITCH), :], f32)
                     for dd in (d, d + DH // 2) for buf in (tbuf, tbuf2))
            for k, term in enumerate(_rhs_terms(*quads)):
                wo7[k, j, pl.ds(d * H, H), :] = term.astype(bf16)

    def ffn_terms(w):
        raw, sums = w
        per = raw.shape[1] // WR

        def body(i):
            p, rs = i // per, _block(i % per, WR)
            quads = (raw[q, rs, _block(p, 128)].astype(f32) for q in range(4))
            for k, term in enumerate(_rhs_terms(*quads)):
                if k in SUM_SLOT:
                    sums[SUM_SLOT[k], p, rs, :] = term.astype(bf16)
        _loop(sums.shape[1] * per, body, WU)

    def panels(w, k, first, count):
        return jnp.concatenate([w[k, first + p] for p in range(count)], axis=1)

    def ffn_rhs(w, k, c0, cols):
        raw, sums = w
        if k in SUM_SLOT:
            return panels(sums, SUM_SLOT[k], c0 // 128, cols // 128)
        return raw[0 if k == 1 else 3, :, pl.ds(c0, cols)]

    def store_lhs(dst, rs, top, bot):
        terms = _lhs_terms(top[:, :DHALF], top[:, DHALF:], bot[:, :DHALF], bot[:, DHALF:])
        for k, term in enumerate(terms):
            dst[k, rs, :] = term.astype(bf16)

    def resid(u, r, rows, cs=slice(None)):
        first = xin[_block((u & (NT - 1)) * (TM // rows) + r, rows), cs].astype(f32)
        if isinstance(u, int):
            return first
        return jnp.where(u < NT, first, xs[u & (NT - 1), _block(r, rows), cs])

    def ln_attn(u, r, rows):
        top, bot = (_ln(resid(u, k, rows)) for k in (r, TH // rows + r))
        store_lhs(xa.at[u & 1], _block(r, rows), top, bot)

    def ln_ffn(tile, r, rows):
        top, bot = (_ln(xs[tile, _block(k, rows), :]) for k in (r, TH // rows + r))
        store_lhs(xf, _block(r, rows), top, bot)

    def halo_carry(dst, src):
        for j in range(NB, 3 * NB):
            dst[j, pl.ds(0, HALO), :] = src[j, pl.ds(TM, HALO), :]

    def halo_init(buf, tile):
        for j in range(NB, 3 * NB):
            first = jnp.broadcast_to(buf[j, pl.ds(HALO, 1), :], (HALO, 128))
            buf[j, pl.ds(0, HALO), :] = jnp.where(tile == 0, first, buf[j, pl.ds(0, HALO), :])

    def attend(buf, tile, r, rows):
        static = isinstance(r, int)
        r0 = r * rows if static else pl.multiple_of(r * rows, rows)
        logits = [None] * W
        for j in range(NB):
            q = buf[j, pl.ds(r0 + HALO, rows), :]
            for w in range(W):
                qk = q * buf[NB + j, pl.ds(r0 + HALO - DIL * w, rows), :]
                logits[w] = qk if j == 0 else logits[w] + qk
        for w in range(W):
            a = logits[w]
            a = a + pltpu.roll(a, 2 * H, 1)
            a = (a + pltpu.roll(a, H, 1)) * SCALE
            if not static or r0 < DIL * w:
                pos = tile * TM + r0 + jax.lax.broadcasted_iota(jnp.int32, (rows, 128), 0)
                a = jnp.where(pos >= DIL * w, a, NEG)
            logits[w] = a
        mx = functools.reduce(jnp.maximum, logits)
        e = [jnp.exp(a - mx) for a in logits]
        inv = 1.0 / functools.reduce(jnp.add, e)
        out = []
        for j in range(NB):
            acc = None
            for w in range(W):
                pv = e[w] * buf[2 * NB + j, pl.ds(r0 + HALO - DIL * w, rows), :]
                acc = pv if acc is None else acc + pv
            out.append(acc * inv)
        return jnp.concatenate(out, axis=1)

    def attention(buf, tile, r, rows):
        store_lhs(ab, _block(r, rows), attend(buf, tile, r, rows), attend(buf, tile, TH // rows + r, rows))

    def qkv_first(c, m):
        res = _dot(x0[:, _block(c, KC)], wqkv[_block(c, KC), _block(m, D)])
        for j in range(NB):
            dst = (m * NB + j, pl.ds(HALO, TM), slice(None))
            part = res[:, j * 128:(j + 1) * 128]
            qkv0[dst] = jnp.where(c == 0, part, qkv0[dst] + part)

    def qkv_proj(slot, c, cols):
        count = cols // 128
        out = _strassen(lambda k: _dot(xa[slot, k], panels(wqkv7, k, c * count, count)))
        for j in range(count):
            p = c * count + j
            slab = (p // (NB // 2)) * NB + p % (NB // 2)
            for i, o in enumerate(out):
                qkv[slot, slab + (i % 2) * (NB // 2), pl.ds(HALO + (i // 2) * TH, TH), :] = o[:, j * 128:(j + 1) * 128]

    def out_proj(u):
        out = _strassen(lambda k: _dot(ab[k], panels(wo7, k, 0, NB // 2)))
        for i, o in enumerate(out):
            cs = _block(i % 2, DHALF)
            xs[u & (NT - 1), _block(i // 2, TH), cs] = resid(u, i // 2, TH, cs) + o

    def ffn_up(c0, cols):
        up = _strassen(lambda k: _dot(xf[k], ffn_rhs(w3, k, c0, cols)))
        gate = _strassen(lambda k: _dot(xf[k], ffn_rhs(w1, k, c0, cols)))
        hidden = []
        for g, u in zip(gate, up):
            half = 0.5 * g
            hidden.append((half * jnp.tanh(half) + half) * u)
        for k, term in enumerate(_lhs_terms(*hidden)):
            hb[k, :, pl.ds(c0, cols)] = term.astype(bf16)

    def ffn_down(tile, c0, cols):
        out = _strassen(lambda k: _dot(hb[k], ffn_rhs(w2, k, c0, cols)))
        for i, o in enumerate(out):
            rs, cs = _block(i // 2, TH), pl.ds((i % 2) * DHALF + c0, cols)
            y = xs[tile, rs, cs] + o
            xs[tile, rs, cs] = y
            ob[rs, cs] = y.astype(ob.dtype)

    x_copies[0].start()
    qkv_copy(0).start()
    x_copies[0].wait()
    for i in range(1, INFLIGHT):
        qkv_copy(i).start()

    def ln_first(r):
        x0[_block(r, LR0), :] = _ln(resid(0, r, LR0)).astype(bf16)
    _loop(TM // LR0, ln_first)

    def first_piece(i):
        @pl.when(i < NPC)
        def _():
            qkv_copy(i).wait()

        @pl.when(i + INFLIGHT < NPC)
        def _():
            qkv_copy(i + INFLIGHT).start()

        @pl.when(i + INFLIGHT == NPC)
        def _():
            x_copies[1].start()

        @pl.when(i == NPC - 1)
        def _():
            wo_copy.start()
        prev = jnp.maximum(i - 1, 0)
        qkv_first(prev // 3, prev % 3)
        permute_qkv(jnp.minimum(i // 3, D // KC - 1), i // 3, i % 3)
    _loop(NPC + 1, first_piece)

    halo_init(qkv0, 0)
    halo_carry(qkv.at[1], qkv0)
    x_copies[1].wait()
    for cp in w3_copies + w1_copies:
        cp.start()
    _loop(TM // LR0, lambda r: ln_attn(1, r, LR0 // 2))
    qkv_terms()

    def second_piece(r):
        attention(qkv0, 0, r, R0)
        qkv_proj(1, r, 3 * DHALF // (TH // R0))
        ln_attn(2, r, R0)
    _loop(TH // R0, second_piece)
    wo_copy.wait()
    _loop(NB // 2, wo_terms)

    def step(u):
        tile, ahead = u & (NT - 1), (u + 1) & (NT - 1)
        s0, s1 = u & 1, (u + 1) & 1

        @pl.when(u + 2 < NU)
        def _():
            halo_carry(qkv.at[s0], qkv.at[s1])
            out_proj(u)
            chunks = 3 * DHALF // PROJ_COLS
            for c in range(chunks):
                qkv_proj(s0, c, PROJ_COLS)
                for r in _share(NR, c, c + 1, chunks):
                    ln_ffn(tile, r, R)

        @pl.when(u + 2 >= NU)
        def _():
            out_proj(u)
            _loop(TM // LR0, lambda r: ln_ffn(tile, r, LR0 // 2))

        @pl.when(u == 0)
        def _():
            for cp in w3_copies:
                cp.wait()
            ffn_terms(w3)
            for cp in w1_copies:
                cp.wait()
            x_copies[2].start()
            for cp in w2_copies:
                cp.start()
            ffn_terms(w1)

        @pl.when(u == 1)
        def _():
            x_copies[2].wait()

        @pl.when(u > NU - NT)
        def _():
            out_copy(tile - 1).wait()

        halo_init(qkv.at[s1], ahead)
        c0 = 0
        for cols in UP_COLS:
            ffn_up(c0, cols)
            for r in _share(NR, c0, c0 + cols, FH):
                attention(qkv.at[s1], ahead, r, R)
            for r in _share(NR, c0, c0 + cols, FH):
                ln_attn(u + 3, r, R)
            c0 += cols

        @pl.when(u == 0)
        def _():
            for cp in w2_copies:
                cp.wait()
            ffn_terms(w2)

        for c0 in range(0, DHALF, DOWN_COLS):
            ffn_down(tile, c0, DOWN_COLS)

        @pl.when(u >= NU - NT)
        def _():
            out_copy(tile).start()

    _loop(NU, step)
    out_copy(NT - 1).wait()


def _ffn_scratch(kh, nh):
    return (pltpu.VMEM((4, kh, nh), bf16),
            pltpu.VMEM((5, nh // 128, kh, 128), bf16))


@jax.jit
def pallas_interleave_layers__sliding_local_dilated__glu_gated_swiglu__prompt_kernel(
    A_x: jax.Array,
    A_wqkv: jax.Array,
    A_wo: jax.Array,
    B_x: jax.Array,
    B_w1: jax.Array,
    B_w3: jax.Array,
    B_w2: jax.Array,
):
    del B_x
    hbm = pl.BlockSpec(memory_space=pl.ANY)
    out = pl.pallas_call(
        _kernel,
        in_specs=[hbm] * 6,
        out_specs=hbm,
        out_shape=jax.ShapeDtypeStruct((S, D), bf16),
        scratch_shapes=[
            pltpu.VMEM((S, D), bf16),
            pltpu.VMEM((D + KC, 3 * D), bf16),
            pltpu.VMEM((D, D), bf16),
            pltpu.VMEM((7, 3 * NB // 2, DHALF, 128), bf16),
            pltpu.VMEM((7, NB // 2, DHALF, 128), bf16),
            _ffn_scratch(DHALF, FH), _ffn_scratch(DHALF, FH), _ffn_scratch(FH, DHALF),
            pltpu.VMEM((H * 40, 128), jnp.uint32),
            pltpu.VMEM((H * 40, 128), jnp.uint32),
            pltpu.VMEM((NT, TM, D), f32),
            pltpu.VMEM((2, 3 * NB, TM + HALO, 128), f32),
            pltpu.VMEM((3 * NB, TM + HALO, 128), f32),
            pltpu.VMEM((TM, D), bf16),
            pltpu.VMEM((2, 7, TH, DHALF), bf16),
            pltpu.VMEM((7, TH, DHALF), bf16),
            pltpu.VMEM((7, TH, DHALF), bf16),
            pltpu.VMEM((7, TH, FH), bf16),
            pltpu.VMEM((TM, D), bf16),
            pltpu.SemaphoreType.DMA((NPC + 17,)),
        ],
        compiler_params=pltpu.CompilerParams(
            vmem_limit_bytes=120 * 1024 * 1024,
            flags={"XLA_TPU_EVENLY_DISTRIBUTE_CRITICAL_NODES": True},
        ),
    )(A_x.reshape(S, D), A_wqkv, A_wo, B_w1, B_w3, B_w2)
    return out.reshape(A_x.shape)
```
